```python
import jax
import jax.numpy as jnp

def _softmax(x, axis=-1):
    return jax.nn.softmax(x, axis=axis)
def _gelu(x):
    return jax.nn.gelu(x, approximate=True)
def _silu(x):
    return jax.nn.silu(x)
def _sigmoid(x):
    return jax.nn.sigmoid(x)
def _layernorm(x, axis=-1, eps=1e-5):
    m = jnp.mean(x, axis=axis, keepdims=True)
    v = jnp.var(x, axis=axis, keepdims=True)
    return (x - m) / jnp.sqrt(v + eps)
def _scatter_add(tgt, idx, src, axis=0):
    return tgt.at[idx].add(src)
def _segment_sum(src, seg, n):
    return jax.ops.segment_sum(src, seg, n)
class _Rng:
    def __init__(self, key):
        self._k = key
    def _next(self):
        self._k, sub = jax.random.split(self._k)
        return sub
    def normal(self, shape):
        return jax.random.normal(self._next(), shape, dtype=jnp.bfloat16)
    def randint(self, lo, hi, shape):
        return jax.random.randint(self._next(), shape, lo, hi, dtype=jnp.int32)
    def uniform(self, shape, lo=0.0, hi=1.0):
        return jax.random.uniform(self._next(), shape, jnp.bfloat16, lo, hi)
    def permutation(self, n):
        return jax.random.permutation(self._next(), n)


kernel_name = 'concat_heads__compressed_kv_cla__spectral_gfnet__prompt'

def setup_inputs():
    _rng = _Rng(jax.random.key(int.from_bytes(__import__("os").urandom(4), "little")))
    _w = (lambda a: (lambda t: t.astype(jnp.bfloat16) if jnp.issubdtype(t.dtype, jnp.floating) else t)(jnp.asarray(a)))
    def _A_setup():
        B, H, Sq, Sk, D, M = 1, 32, 2048, 2048, 128, 1024
        Dc = 4 * D
        return {
            "x": _w((lambda *s: _rng.normal(s) * 0.05)(B, Sq, M)),
            "c_kv": _w((lambda *s: _rng.normal(s) * 0.05)(B, Sk, Dc)),
            "w_q": _w((lambda *s: _rng.normal(s) * 0.05)(M, H, D) * (M ** -0.5)),
            "w_uk": _w((lambda *s: _rng.normal(s) * 0.05)(Dc, H, D) * (Dc ** -0.5)),
            "w_uv": _w((lambda *s: _rng.normal(s) * 0.05)(Dc, H, D) * (Dc ** -0.5)),
            "w_o": _w((lambda *s: _rng.normal(s) * 0.05)(H, D, M) * ((H * D) ** -0.5)),
        }
    _A_in = _A_setup()

    def _B_setup():
        B, S, D = 1, 2048, 1024
        Df = D // 2 + 1
        return {
            "x": _w((lambda *s: _rng.normal(s) * 0.05)(B, S, D)),
            "w_r": _w((lambda *s: _rng.normal(s) * 0.05)(S, Df) * 0.02),
            "w_i": _w((lambda *s: _rng.normal(s) * 0.05)(S, Df) * 0.02),
        }
    _B_in = _B_setup()

    return {
        "A_x": _A_in["x"],
        "A_c_kv": _A_in["c_kv"],
        "A_w_q": _A_in["w_q"],
        "A_w_uk": _A_in["w_uk"],
        "A_w_uv": _A_in["w_uv"],
        "A_w_o": _A_in["w_o"],
        "B_x": _B_in["x"],
        "B_w_r": _B_in["w_r"],
        "B_w_i": _B_in["w_i"],
    }

def reference(A_x, A_c_kv, A_w_q, A_w_uk, A_w_uv, A_w_o, B_x, B_w_r, B_w_i):
    def _A_ref(x, c_kv, w_q, w_uk, w_uv, w_o):
        B, Sq, M = x.shape[0], x.shape[1], x.shape[2]
        Sk = c_kv.shape[1]
        H, D = w_q.shape[1], w_q.shape[2]
        q = jnp.einsum("bqm,mhd->bhqd", x, w_q)
        k = jnp.einsum("bkc,chd->bhkd", c_kv, w_uk)
        v = jnp.einsum("bkc,chd->bhkd", c_kv, w_uv)
        scores = jnp.einsum("bhqd,bhkd->bhqk", q, k) * (D ** -0.5)
        off = Sk - Sq
        qi = jnp.arange(Sq)[:, None]
        kj = jnp.arange(Sk)[None, :]
        cmask = kj <= (qi + off)
        scores = jnp.where(cmask[None, None], scores, -1e9)
        p = _softmax(scores, axis=-1)
        ctx = jnp.einsum("bhqk,bhkd->bhqd", p, v)
        return jnp.einsum("bhqd,hdm->bqm", ctx, w_o)

    def _B_ref(x, w_r, w_i):
        B, S, D = x.shape
        X = (lambda x, axes=(-2,-1): jnp.fft.rfft2(x.astype(jnp.float32), axes=axes))(x, axes=(-2, -1))
        W = w_r + 1j * w_i
        X = X * W
        y = (lambda x, s, axes=(-2,-1): jnp.fft.irfft2(x, s=s, axes=axes).astype(jnp.bfloat16))(X, (S, D), axes=(-2, -1))
        return y

    a = _A_ref(A_x, A_c_kv, A_w_q, A_w_uk, A_w_uv, A_w_o)
    b = _B_ref(B_x, B_w_r, B_w_i)
    return jnp.concatenate([a, b], axis=-1)
```

```python
import functools
import math

import jax
import jax.numpy as jnp
import jax.experimental.pallas as pl
import jax.experimental.pallas.tpu as pltpu
import ml_dtypes
import numpy as np
from jax import lax

SEQ = 2048
D = 128
H = 32
M = 1024
DC = 512
SB = 2048
DB = 1024
DF = DB // 2 + 1
N1 = 128
N2 = 16
UR = 528
VR = 640
NT = (((1,), (1,)), ((), ()))
QSCALE = (D ** -0.5) * math.log2(math.e)
L_LO = 2.0 ** -30
L_HI = 2.0 ** 30
HI16 = 0xFFFF0000


@functools.lru_cache(maxsize=None)
def _dft_consts():
    th = 2 * np.pi / DB
    d = np.arange(256, dtype=np.float64) + 0.5
    m = np.arange(256, dtype=np.float64)
    fe, fo = 2 * m, 2 * m + 1
    sny = np.zeros((16, 256))
    sny[0] = -np.sin(th * 512 * d)
    dfw = np.concatenate([np.cos(th * np.outer(fe, d)), np.cos(th * np.outer(fo, d)),
                          -np.sin(th * np.outer(fe, d)), sny, -np.sin(th * np.outer(fo, d))], 0)
    cfe = np.full(256, 2.0 / DB)
    cfe[0] = 1.0 / DB
    cfo = np.full(256, 2.0 / DB)
    gse = cfe[:, None] * np.sin(th * np.outer(fe, d))
    gse[0] = (1.0 / DB) * np.sin(th * 512 * d)
    dinv = np.stack([cfe[:, None] * np.cos(th * np.outer(fe, d)),
                     cfo[:, None] * np.cos(th * np.outer(fo, d)),
                     gse, cfo[:, None] * np.sin(th * np.outer(fo, d))], 0)
    n2 = np.arange(N2)[:, None, None]
    n1 = np.arange(N1)[None, :, None]
    k1 = np.arange(N1)[None, None, :]
    ang = -2 * np.pi * k1 * (N2 * n1 + n2) / SB
    fr, fi = np.cos(ang), np.sin(ang)
    fm = np.concatenate([np.concatenate([fr, fi], 2), np.concatenate([-fi, fr], 2)], 1)
    gr, gi = fr / SB, -fi / SB
    gm = np.concatenate([np.concatenate([gr, -gi], 2), np.concatenate([gi, gr], 2)], 1)
    bf = ml_dtypes.bfloat16
    return tuple(np.asarray(a, dtype=np.float32).astype(bf) for a in (dfw, dinv, fm, gm))


def _cmul_const(xr, xi, ang):
    c, s = math.cos(ang), math.sin(ang)
    eps = 1e-9
    if abs(s) < eps:
        return (xr, xi) if c > 0 else (-xr, -xi)
    if abs(c) < eps:
        return (-xi, xr) if s > 0 else (xi, -xr)
    if abs(abs(c) - abs(s)) < eps:
        if c * s > 0:
            return (xr - xi) * c, (xr + xi) * c
        return (xr + xi) * c, (xi - xr) * c
    return xr * c - xi * s, xr * s + xi * c


def _fft(xs, sign):
    n = len(xs)
    if n == 1:
        return xs
    if n == 2:
        (ar, ai), (br, bi) = xs
        return [(ar + br, ai + bi), (ar - br, ai - bi)]
    if n == 4:
        (ar, ai), (br, bi), (cr, ci), (dr, di) = xs
        t0r, t0i = ar + cr, ai + ci
        t1r, t1i = ar - cr, ai - ci
        t2r, t2i = br + dr, bi + di
        t3r, t3i = br - dr, bi - di
        if sign > 0:
            return [(t0r + t2r, t0i + t2i), (t1r - t3i, t1i + t3r),
                    (t0r - t2r, t0i - t2i), (t1r + t3i, t1i - t3r)]
        return [(t0r + t2r, t0i + t2i), (t1r + t3i, t1i - t3r),
                (t0r - t2r, t0i - t2i), (t1r - t3i, t1i + t3r)]
    ev = _fft(xs[0::2], sign)
    od = _fft(xs[1::2], sign)
    out = [None] * n
    for k in range(n // 2):
        er, ei = ev[k]
        if k * 4 == n:
            o_r, o_i = od[k]
            if sign > 0:
                out[k] = (er - o_i, ei + o_r)
                out[k + n // 2] = (er + o_i, ei - o_r)
            else:
                out[k] = (er + o_i, ei - o_r)
                out[k + n // 2] = (er - o_i, ei + o_r)
        else:
            tr, ti = _cmul_const(od[k][0], od[k][1], sign * 2 * math.pi * k / n)
            out[k] = (er + tr, ei + ti)
            out[k + n // 2] = (er - tr, ei - ti)
    return out


def _unpack_head(wbuf, e):
    sh = (16 * (1 - e)).astype(jnp.uint32)
    w = pltpu.bitcast((wbuf[...] << sh) & jnp.uint32(HI16), jnp.float32)
    return w.astype(jnp.bfloat16)


def _attn_plan(qi, bq, bk, stair):
    r0 = qi * bq
    steps = []
    c = 0
    while c + bk <= r0:
        steps.append((0, c, bk))
        c += bk
    if c < r0:
        steps.append((0, c, r0 - c))
    for t in range(bq // stair):
        steps.append((t * stair, r0 + t * stair, stair))
    return steps


def _attn_fast(q_ref, k_ref, v_ref, o_ref, bq=512, bk=512, stair=128):
    R = 128
    row = lax.broadcasted_iota(jnp.int32, (R, 128), 0)
    col = lax.broadcasted_iota(jnp.int32, (R, 128), 1)
    tri = col <= row
    bad = jnp.zeros((8, 128), jnp.int32)
    for qi in range(SEQ // bq):
        r0 = qi * bq
        nsub = bq // R
        acc = [None] * nsub
        lv = [None] * nsub
        for (roff, c0, clen) in _attn_plan(qi, bq, bk, stair):
            mr = bq - roff
            q = q_ref[pl.ds(r0 + roff, mr), :]
            k = k_ref[pl.ds(c0, clen), :]
            v = v_ref[pl.ds(c0, clen), :]
            s = lax.dot_general(q, k, NT, preferred_element_type=jnp.float32)
            p = jnp.exp2(s)
            if c0 + clen - 1 > r0 + roff:
                rows = []
                for a in range(mr // R):
                    ra = r0 + roff + a * R
                    cols = []
                    for b in range(clen // 128):
                        cb = c0 + b * 128
                        t = p[a * R:(a + 1) * R, b * 128:(b + 1) * 128]
                        if cb == ra:
                            t = jnp.where(tri, t, 0.0)
                        elif cb > ra:
                            t = jnp.zeros_like(t)
                        cols.append(t)
                    rows.append(jnp.concatenate(cols, axis=1) if len(cols) > 1 else cols[0])
                p = jnp.concatenate(rows, axis=0) if len(rows) > 1 else rows[0]
            pv = jnp.dot(p.astype(jnp.bfloat16), v, preferred_element_type=jnp.float32)
            for a in range(mr // R):
                ia = roff // R + a
                pa = p[a * R:(a + 1) * R, :]
                ps = pa[:, 0:128]
                for b in range(1, clen // 128):
                    ps = ps + pa[:, b * 128:(b + 1) * 128]
                lv[ia] = ps if lv[ia] is None else lv[ia] + ps
                t = pv[a * R:(a + 1) * R, :]
                acc[ia] = t if acc[ia] is None else acc[ia] + t
        for a in range(nsub):
            l = jnp.sum(lv[a], axis=-1, keepdims=True)
            o = acc[a] * (1.0 / l)
            ok = (l >= L_LO) & (l <= L_HI) & (jnp.abs(o) <= 3.0e38)
            nb = jnp.where(ok, 0, 1).astype(jnp.int32)
            for i in range(R // 8):
                bad = jnp.maximum(bad, nb[i * 8:(i + 1) * 8, :])
            o_ref[pl.ds(r0 + a * R, R), :] = o.astype(o_ref.dtype)
    return bad


def _attn_exact(q_ref, k_ref, v_ref, o_ref, bq=256, bk=256):
    scale = D ** -0.5

    def q_body(qi, carry):
        rs = pl.ds(pl.multiple_of(qi * bq, bq), bq)
        q = q_ref[rs, :]

        def k_body(kj, st):
            m, l, acc = st
            ks = pl.ds(pl.multiple_of(kj * bk, bk), bk)
            s = lax.dot_general(q, k_ref[ks, :], NT, preferred_element_type=jnp.float32) * scale
            row = lax.broadcasted_iota(jnp.int32, (bq, bk), 0) + qi * bq
            col = lax.broadcasted_iota(jnp.int32, (bq, bk), 1) + kj * bk
            s = jnp.where(col <= row, s, -1e9)
            m_new = jnp.maximum(m, jnp.max(s, axis=-1, keepdims=True))
            p = jnp.exp(s - m_new)
            alpha = jnp.exp(m - m_new)
            l = alpha * l + jnp.sum(p, axis=-1, keepdims=True)
            acc = alpha * acc + jnp.dot(p.astype(jnp.bfloat16), v_ref[ks, :],
                                        preferred_element_type=jnp.float32)
            return m_new, l, acc

        init = (jnp.full((bq, 1), -jnp.inf, jnp.float32), jnp.zeros((bq, 1), jnp.float32),
                jnp.zeros((bq, D), jnp.float32))
        m, l, acc = lax.fori_loop(0, SEQ // bk, k_body, init)
        o_ref[rs, :] = (acc / l).astype(o_ref.dtype)
        return carry

    lax.fori_loop(0, SEQ // bq, q_body, 0)


def _unpack2(u):
    return (pltpu.bitcast(u << 16, jnp.float32), pltpu.bitcast(u & jnp.uint32(HI16), jnp.float32))


def _b_stage1(j, xb, dfw_ref, fm_ref, tv):
    ridx = 127 - lax.broadcasted_iota(jnp.int32, (N1, 128), 1)
    q0, q1r, q2, q3r = [], [], [], []
    for t in range(2):
        q0.append(_unpack2(xb[j, :, pl.ds(t * 128, 128)]))
        q1r.append(_unpack2(jnp.take_along_axis(xb[j, :, pl.ds((3 - t) * 128, 128)], ridx, axis=1)))
        q2.append(_unpack2(xb[j, :, pl.ds((4 + t) * 128, 128)]))
        q3r.append(_unpack2(jnp.take_along_axis(xb[j, :, pl.ds((7 - t) * 128, 128)], ridx, axis=1)))
    for e in range(2):
        n2 = 2 * j + e
        ee, eo, oe, oo = [], [], [], []
        for t in range(2):
            x0, r1, x2, r3 = q0[t][e], q1r[t][e], q2[t][e], q3r[t][e]
            a = x0 + r3
            b = x0 - r3
            c = r1 + x2
            dd = r1 - x2
            ee.append((a + c).astype(jnp.bfloat16))
            eo.append((a - c).astype(jnp.bfloat16))
            oe.append((b - dd).astype(jnp.bfloat16))
            oo.append((b + dd).astype(jnp.bfloat16))
        ee, eo, oe, oo = (jnp.concatenate(z, axis=1) for z in (ee, eo, oe, oo))
        ur_e = lax.dot_general(dfw_ref[pl.ds(0, 256), :], ee, NT, preferred_element_type=jnp.float32)
        ur_o = lax.dot_general(dfw_ref[pl.ds(256, 256), :], eo, NT, preferred_element_type=jnp.float32)
        ui_en = lax.dot_general(dfw_ref[pl.ds(512, 272), :], oe, NT, preferred_element_type=jnp.float32)
        ui_o = lax.dot_general(dfw_ref[pl.ds(784, 256), :], oo, NT, preferred_element_type=jnp.float32)
        ur = jnp.concatenate([ur_e, ur_o, jnp.zeros((16, 128), jnp.float32)], axis=0)
        ui = jnp.concatenate([ui_en[:256], ui_o, ui_en[256:]], axis=0)
        u = jnp.concatenate([ur, ui], axis=1).astype(jnp.bfloat16)
        tv[n2, pl.ds(0, UR), :] = jnp.dot(u, fm_ref[n2], preferred_element_type=jnp.float32)


def _b_stage2(g, kind, tv, wru, wiu, wr_v, wi_v):
    r0 = 512 if kind == 2 else pl.multiple_of(kind * 256 + g * 8, 8)
    xs = [(tv[n2, pl.ds(r0, 8), pl.ds(0, 128)], tv[n2, pl.ds(r0, 8), pl.ds(128, 128)])
          for n2 in range(N2)]
    ys = _fft(xs, -1)
    zs = []
    for k2 in range(N2):
        cs = pl.ds(k2 * 128, 128)
        if kind == 2:
            wr = jnp.broadcast_to(wr_v[pl.ds(512, 1), cs].astype(jnp.float32), (8, 128))
            wi = jnp.broadcast_to(wi_v[pl.ds(512, 1), cs].astype(jnp.float32), (8, 128))
        else:
            g8 = pl.ds(pl.multiple_of(g * 8, 8), 8)
            wr = _unpack2(wru[g8, cs])[kind]
            wi = _unpack2(wiu[g8, cs])[kind]
        xr, xi = ys[k2]
        zs.append((xr * wr - xi * wi, xr * wi + xi * wr))
    vs = _fft(zs, +1)
    for n2 in range(N2):
        tv[n2, pl.ds(r0, 8), pl.ds(0, 128)] = vs[n2][0]
        tv[n2, pl.ds(r0, 8), pl.ds(128, 128)] = vs[n2][1]


def _b_stage3(j, tv, gm_ref, dinv_ref):
    lane = lax.broadcasted_iota(jnp.int32, (N1, 128), 1)
    ridx = 127 - lax.broadcasted_iota(jnp.int32, (N1, 128), 1)
    zr, zi = [], []
    for e in range(2):
        n2 = 2 * j + e
        v = tv[n2].astype(jnp.bfloat16)
        zt = lax.dot_general(gm_ref[n2], v, NT, preferred_element_type=jnp.float32)
        zr.append(zt[:128, :512].astype(jnp.bfloat16))
        zi0 = jnp.where(lane == 0, zt[128:, 512:640], zt[128:, 0:128])
        zi.append(jnp.concatenate([zi0, zt[128:, 128:512]], axis=1).astype(jnp.bfloat16))
    zr = jnp.concatenate(zr, axis=0)
    zi = jnp.concatenate(zi, axis=0)
    pe = jnp.dot(zr[:, :256], dinv_ref[0], preferred_element_type=jnp.float32)
    po = jnp.dot(zr[:, 256:], dinv_ref[1], preferred_element_type=jnp.float32)
    qe = jnp.dot(zi[:, :256], dinv_ref[2], preferred_element_type=jnp.float32)
    qo = jnp.dot(zi[:, 256:], dinv_ref[3], preferred_element_type=jnp.float32)
    ps, pd, qs, qd = pe + po, pe - po, qe + qo, qe - qo
    y0, y1r, y2, y3r = ps - qs, pd + qd, pd - qd, ps + qs

    def pk(y, t):
        return pltpu.pack_elementwise([y[:128, t * 128:(t + 1) * 128], y[128:, t * 128:(t + 1) * 128]],
                                      packed_dtype=jnp.bfloat16)

    outs = [None] * 8
    for t in range(2):
        outs[t] = pk(y0, t)
        outs[3 - t] = jnp.take_along_axis(pk(y1r, t), ridx, axis=1)
        outs[4 + t] = pk(y2, t)
        outs[7 - t] = jnp.take_along_axis(pk(y3r, t), ridx, axis=1)
    return jnp.concatenate(outs, axis=1)


OC = 256


def _kernel(x_hbm, c_hbm, wq_hbm, wk_hbm, wv_hbm, wo_hbm, bx_hbm, wr_hbm, wi_hbm,
            dfw_hbm, dinv_hbm, fm_hbm, gm_hbm, o_hbm,
            x_v, c_v, wq_b, wk_b, wv_b, q_s, k_s, v_s, ctx_s, wo_v, flags, o_st,
            xb, dfw_v, dinv_v, fm_v, gm_v, wr_v, wi_v, wru, wiu, tv, y_st,
            sems, wsem, xsem, osem, ysem):
    wq_u = wq_hbm.bitcast(jnp.uint32)
    wk_u = wk_hbm.bitcast(jnp.uint32)
    wv_u = wv_hbm.bitcast(jnp.uint32)
    bx_u = bx_hbm.bitcast(jnp.uint32)
    o_u = o_hbm.bitcast(jnp.uint32)

    def w_copies(p, slot):
        return [pltpu.make_async_copy(wq_u.at[:, p, :], wq_b.at[slot], wsem.at[slot, 0]),
                pltpu.make_async_copy(wk_u.at[:, p, :], wk_b.at[slot], wsem.at[slot, 1]),
                pltpu.make_async_copy(wv_u.at[:, p, :], wv_b.at[slot], wsem.at[slot, 2])]

    cp_c = pltpu.make_async_copy(c_hbm, c_v, sems.at[0])
    cp_x = pltpu.make_async_copy(x_hbm, x_v, sems.at[1])
    cp_wo = pltpu.make_async_copy(wo_hbm, wo_v, sems.at[2])
    cp_wr = pltpu.make_async_copy(wr_hbm, wr_v, sems.at[3])
    cp_wi = pltpu.make_async_copy(wi_hbm, wi_v, sems.at[4])
    cp_dfw = pltpu.make_async_copy(dfw_hbm, dfw_v, sems.at[5])
    cp_dinv = pltpu.make_async_copy(dinv_hbm, dinv_v, sems.at[6])
    cp_fm = pltpu.make_async_copy(fm_hbm, fm_v, sems.at[7])
    cp_gm = pltpu.make_async_copy(gm_hbm, gm_v, sems.at[8])
    cp_bx = [pltpu.make_async_copy(bx_u.at[:, j, :], xb.at[j], xsem.at[j]) for j in range(N2 // 2)]

    cp_c.start()
    for c in w_copies(0, 0):
        c.start()
    cp_x.start()
    cp_c.wait()
    cp_x.wait()

    def project(wq, wk, wv, qscale):
        rc = 512
        for r in range(SEQ // rc):
            rs = pl.ds(r * rc, rc)
            cblk = c_v[rs, :]
            k_s[rs, :] = jnp.dot(cblk, wk, preferred_element_type=jnp.float32).astype(jnp.bfloat16)
            v_s[rs, :] = jnp.dot(cblk, wv, preferred_element_type=jnp.float32).astype(jnp.bfloat16)
            q = jnp.dot(x_v[rs, :], wq, preferred_element_type=jnp.float32)
            q_s[rs, :] = (q * qscale if qscale is not None else q).astype(jnp.bfloat16)

    def head_body(h, carry):
        p = h // 2
        e = h % 2
        slot = p % 2

        @pl.when(e == 0)
        def _():
            for c in w_copies(p, slot):
                c.wait()

            @pl.when(p + 1 < H // 2)
            def _():
                for c in w_copies(p + 1, 1 - slot):
                    c.start()

        @pl.when(h == 1)
        def _():
            cp_wo.start()

        @pl.when(h == 5)
        def _():
            for c in cp_bx:
                c.start()
            cp_dfw.start()
            cp_dinv.start()

        @pl.when(h == 9)
        def _():
            cp_fm.start()
            cp_gm.start()
            cp_wr.start()
            cp_wi.start()

        project(_unpack_head(wq_b.at[slot], e), _unpack_head(wk_b.at[slot], e),
                _unpack_head(wv_b.at[slot], e), QSCALE)
        flags[h] = _attn_fast(q_s, k_s, v_s, ctx_s.at[h])
        return carry

    lax.fori_loop(0, H, head_body, 0)

    any_bad = jnp.max(flags[...].reshape(H * 8, 128))

    @pl.when(any_bad > 0)
    def _():
        def redo(h, carry):
            @pl.when(jnp.max(flags[h]) > 0)
            def _():
                p = h // 2
                e = h % 2
                for c in w_copies(p, 0):
                    c.start()
                for c in w_copies(p, 0):
                    c.wait()
                project(_unpack_head(wq_b.at[0], e), _unpack_head(wk_b.at[0], e),
                        _unpack_head(wv_b.at[0], e), None)
                _attn_exact(q_s, k_s, v_s, ctx_s.at[h])
            return carry
        lax.fori_loop(0, H, redo, 0)

    n_oc = SEQ // OC
    rpc = OC // N2

    def out_copy(r, slot):
        return pltpu.make_async_copy(o_st.at[slot], o_hbm.at[pl.ds(r * rpc, rpc), :, pl.ds(0, M)],
                                     osem.at[slot])

    cp_wo.wait()

    def oproj_body(r, carry):
        rs = pl.ds(pl.multiple_of(r * OC, OC), OC)
        acc = None
        for hg in range(H // 4):
            lhs = jnp.concatenate([ctx_s[hg * 4 + i, rs, :] for i in range(4)], axis=1)
            rhs = wo_v[pl.ds(hg * 4, 4)].reshape(4 * D, M)
            t = jnp.dot(lhs, rhs, preferred_element_type=jnp.float32)
            acc = t if acc is None else acc + t
        slot = r % 2

        @pl.when(r >= 2)
        def _():
            out_copy(r - 2, slot).wait()

        o_st[slot] = acc.astype(jnp.bfloat16).reshape(rpc, N2, M)
        out_copy(r, slot).start()
        return carry

    lax.fori_loop(0, n_oc, oproj_body, 0)

    for c in cp_bx:
        c.wait()
    cp_dfw.wait()
    cp_fm.wait()
    tv[:, pl.ds(UR, VR - UR), :] = jnp.zeros((N2, VR - UR, 256), jnp.float32)

    def b1_body(j, carry):
        _b_stage1(j, xb, dfw_v, fm_v, tv)
        return carry

    lax.fori_loop(0, N2 // 2, b1_body, 0)
    for r in (n_oc - 2, n_oc - 1):
        out_copy(r, r % 2).wait()
    cp_wr.wait()
    cp_wi.wait()
    wru[...] = pltpu.bitcast(wr_v[pl.ds(0, 512), :], jnp.uint32)
    wiu[...] = pltpu.bitcast(wi_v[pl.ds(0, 512), :], jnp.uint32)

    def b2_body(g, carry):
        _b_stage2(g, 0, tv, wru, wiu, wr_v, wi_v)
        _b_stage2(g, 1, tv, wru, wiu, wr_v, wi_v)
        return carry

    lax.fori_loop(0, 32, b2_body, 0)
    _b_stage2(0, 2, tv, wru, wiu, wr_v, wi_v)
    cp_gm.wait()
    cp_dinv.wait()

    def y_copy(j, slot):
        return pltpu.make_async_copy(y_st.at[slot], o_u.at[:, j, pl.ds(M, DB)], ysem.at[slot])

    def b3_body(j, carry):
        y = _b_stage3(j, tv, gm_v, dinv_v)
        slot = j % 2

        @pl.when(j >= 2)
        def _():
            y_copy(j - 2, slot).wait()

        y_st[slot] = y
        y_copy(j, slot).start()
        return carry

    lax.fori_loop(0, N2 // 2, b3_body, 0)
    for j in (N2 // 2 - 2, N2 // 2 - 1):
        y_copy(j, j % 2).wait()


@jax.jit
def pallas_concat_heads__compressed_kv_cla__spectral_gfnet__prompt_kernel(
    A_x: jax.Array,
    A_c_kv: jax.Array,
    A_w_q: jax.Array,
    A_w_uk: jax.Array,
    A_w_uv: jax.Array,
    A_w_o: jax.Array,
    B_x: jax.Array,
    B_w_r: jax.Array,
    B_w_i: jax.Array,
):
    dfw, dinv, fm, gm = _dft_consts()
    hbm = pl.BlockSpec(memory_space=pltpu.HBM)
    bf16, f32, u32 = jnp.bfloat16, jnp.float32, jnp.uint32
    scratch = [
        pltpu.VMEM((SEQ, M), bf16), pltpu.VMEM((SEQ, DC), bf16),
        pltpu.VMEM((2, M, D), u32), pltpu.VMEM((2, DC, D), u32), pltpu.VMEM((2, DC, D), u32),
        pltpu.VMEM((SEQ, D), bf16), pltpu.VMEM((SEQ, D), bf16), pltpu.VMEM((SEQ, D), bf16),
        pltpu.VMEM((H, SEQ, D), bf16), pltpu.VMEM((H, D, M), bf16),
        pltpu.VMEM((H, 8, 128), jnp.int32),
        pltpu.VMEM((2, OC // N2, N2, M), bf16),
        pltpu.VMEM((N2 // 2, N1, DB), u32),
        pltpu.VMEM(dfw.shape, bf16), pltpu.VMEM(dinv.shape, bf16),
        pltpu.VMEM(fm.shape, bf16), pltpu.VMEM(gm.shape, bf16),
        pltpu.VMEM((DF, SB), bf16), pltpu.VMEM((DF, SB), bf16),
        pltpu.VMEM((256, SB), u32), pltpu.VMEM((256, SB), u32),
        pltpu.VMEM((N2, VR, 256), f32),
        pltpu.VMEM((2, N1, DB), u32),
        pltpu.SemaphoreType.DMA((9,)), pltpu.SemaphoreType.DMA((2, 3)),
        pltpu.SemaphoreType.DMA((N2 // 2,)), pltpu.SemaphoreType.DMA((2,)),
        pltpu.SemaphoreType.DMA((2,)),
    ]
    out = pl.pallas_call(
        _kernel,
        out_shape=jax.ShapeDtypeStruct((N1, N2, M + DB), bf16),
        in_specs=[hbm] * 13,
        out_specs=hbm,
        scratch_shapes=scratch,
        compiler_params=pltpu.CompilerParams(vmem_limit_bytes=120 * 2 ** 20),
    )(A_x.reshape(SEQ, M), A_c_kv.reshape(SEQ, DC), A_w_q, A_w_uk, A_w_uv, A_w_o,
      B_x.reshape(N1, N2, DB), B_w_r.T, B_w_i.T, dfw, dinv, fm, gm)
    return out.reshape(1, SEQ, M + DB)
```

```python
import functools
import math

import jax
import jax.numpy as jnp
import jax.experimental.pallas as pl
import jax.experimental.pallas.tpu as pltpu
import ml_dtypes
import numpy as np
from jax import lax

SEQ = 2048
D = 128
H = 32
M = 1024
DC = 512
SB = 2048
DB = 1024
DF = DB // 2 + 1
N1 = 128
N2 = 16
UR = 528
VR = 640
NT = (((1,), (1,)), ((), ()))
QSCALE = (D ** -0.5) * math.log2(math.e)
L_LO = 2.0 ** -30
L_HI = 2.0 ** 30
HI16 = 0xFFFF0000


@functools.lru_cache(maxsize=None)
def _dft_consts():
    th = 2 * np.pi / DB
    d = np.arange(256, dtype=np.float64) + 0.5
    m = np.arange(256, dtype=np.float64)
    fe, fo = 2 * m, 2 * m + 1
    sny = np.zeros((16, 256))
    sny[0] = -np.sin(th * 512 * d)
    dfw = np.concatenate([np.cos(th * np.outer(fe, d)), np.cos(th * np.outer(fo, d)),
                          -np.sin(th * np.outer(fe, d)), sny, -np.sin(th * np.outer(fo, d))], 0)
    cfe = np.full(256, 2.0 / DB)
    cfe[0] = 1.0 / DB
    cfo = np.full(256, 2.0 / DB)
    gse = cfe[:, None] * np.sin(th * np.outer(fe, d))
    gse[0] = (1.0 / DB) * np.sin(th * 512 * d)
    dinv = np.stack([cfe[:, None] * np.cos(th * np.outer(fe, d)),
                     cfo[:, None] * np.cos(th * np.outer(fo, d)),
                     gse, cfo[:, None] * np.sin(th * np.outer(fo, d))], 0)
    n2 = np.arange(N2)[:, None, None]
    n1 = np.arange(N1)[None, :, None]
    k1 = np.arange(N1)[None, None, :]
    ang = -2 * np.pi * k1 * (N2 * n1 + n2) / SB
    fr, fi = np.cos(ang), np.sin(ang)
    fm = np.concatenate([np.concatenate([fr, fi], 2), np.concatenate([-fi, fr], 2)], 1)
    gr, gi = fr / SB, -fi / SB
    gm = np.concatenate([np.concatenate([gr, -gi], 2), np.concatenate([gi, gr], 2)], 1)
    bf = ml_dtypes.bfloat16
    return tuple(np.asarray(a, dtype=np.float32).astype(bf) for a in (dfw, dinv, fm, gm))


def _cmul_const(xr, xi, ang):
    c, s = math.cos(ang), math.sin(ang)
    eps = 1e-9
    if abs(s) < eps:
        return (xr, xi) if c > 0 else (-xr, -xi)
    if abs(c) < eps:
        return (-xi, xr) if s > 0 else (xi, -xr)
    if abs(abs(c) - abs(s)) < eps:
        if c * s > 0:
            return (xr - xi) * c, (xr + xi) * c
        return (xr + xi) * c, (xi - xr) * c
    return xr * c - xi * s, xr * s + xi * c


def _fft(xs, sign):
    n = len(xs)
    if n == 1:
        return xs
    if n == 2:
        (ar, ai), (br, bi) = xs
        return [(ar + br, ai + bi), (ar - br, ai - bi)]
    if n == 4:
        (ar, ai), (br, bi), (cr, ci), (dr, di) = xs
        t0r, t0i = ar + cr, ai + ci
        t1r, t1i = ar - cr, ai - ci
        t2r, t2i = br + dr, bi + di
        t3r, t3i = br - dr, bi - di
        if sign > 0:
            return [(t0r + t2r, t0i + t2i), (t1r - t3i, t1i + t3r),
                    (t0r - t2r, t0i - t2i), (t1r + t3i, t1i - t3r)]
        return [(t0r + t2r, t0i + t2i), (t1r + t3i, t1i - t3r),
                (t0r - t2r, t0i - t2i), (t1r - t3i, t1i + t3r)]
    ev = _fft(xs[0::2], sign)
    od = _fft(xs[1::2], sign)
    out = [None] * n
    for k in range(n // 2):
        er, ei = ev[k]
        if k * 4 == n:
            o_r, o_i = od[k]
            if sign > 0:
                out[k] = (er - o_i, ei + o_r)
                out[k + n // 2] = (er + o_i, ei - o_r)
            else:
                out[k] = (er + o_i, ei - o_r)
                out[k + n // 2] = (er - o_i, ei + o_r)
        else:
            tr, ti = _cmul_const(od[k][0], od[k][1], sign * 2 * math.pi * k / n)
            out[k] = (er + tr, ei + ti)
            out[k + n // 2] = (er - tr, ei - ti)
    return out


def _unpack_head(wbuf, e):
    sh = (16 * (1 - e)).astype(jnp.uint32)
    w = pltpu.bitcast((wbuf[...] << sh) & jnp.uint32(HI16), jnp.float32)
    return w.astype(jnp.bfloat16)


def _strassen_rhs(b11, b12, b21, b22):
    bf = jnp.bfloat16
    return [(b11 + b22).astype(bf), b11.astype(bf), (b12 - b22).astype(bf), (b21 - b11).astype(bf),
            b22.astype(bf), (b11 + b12).astype(bf), (b21 + b22).astype(bf)]


def _strassen_lhs(a11, a12, a21, a22):
    bf = jnp.bfloat16
    f11, f12, f21, f22 = (a.astype(jnp.float32) for a in (a11, a12, a21, a22))
    return [(f11 + f22).astype(bf), (f21 + f22).astype(bf), a11, a22,
            (f11 + f12).astype(bf), (f21 - f11).astype(bf), (f12 - f22).astype(bf)]


def _strassen_out(lhs, rhs):
    m1, m2, m3, m4, m5, m6, m7 = (jnp.dot(a, b, preferred_element_type=jnp.float32)
                                  for a, b in zip(lhs, rhs))
    return m1 + m4 - m5 + m7, m3 + m5, m2 + m4, m1 - m2 + m3 + m6


def _attn_plan(qi, bq, bk, stair):
    r0 = qi * bq
    steps = []
    c = 0
    while c + bk <= r0:
        steps.append((0, c, bk))
        c += bk
    if c < r0:
        steps.append((0, c, r0 - c))
    for t in range(bq // stair):
        steps.append((t * stair, r0 + t * stair, stair))
    return steps


def _attn_fast(q_ref, k_ref, v_ref, o_ref, fill=None, bq=512, bk=512, stair=128):
    R = 128
    row = lax.broadcasted_iota(jnp.int32, (R, 128), 0)
    col = lax.broadcasted_iota(jnp.int32, (R, 128), 1)
    tri = col <= row
    bad = jnp.zeros((8, 128), jnp.int32)
    for qi in range(SEQ // bq):
        r0 = qi * bq
        nsub = bq // R
        acc = [None] * nsub
        lv = [None] * nsub
        for (roff, c0, clen) in _attn_plan(qi, bq, bk, stair):
            mr = bq - roff
            q = q_ref[pl.ds(r0 + roff, mr), :]
            k = k_ref[pl.ds(c0, clen), :]
            v = v_ref[pl.ds(c0, clen), :]
            s = lax.dot_general(q, k, NT, preferred_element_type=jnp.float32)
            p = jnp.exp2(s)
            if c0 + clen - 1 > r0 + roff:
                rows = []
                for a in range(mr // R):
                    ra = r0 + roff + a * R
                    cols = []
                    for b in range(clen // 128):
                        cb = c0 + b * 128
                        t = p[a * R:(a + 1) * R, b * 128:(b + 1) * 128]
                        if cb == ra:
                            t = jnp.where(tri, t, 0.0)
                        elif cb > ra:
                            t = jnp.zeros_like(t)
                        cols.append(t)
                    rows.append(jnp.concatenate(cols, axis=1) if len(cols) > 1 else cols[0])
                p = jnp.concatenate(rows, axis=0) if len(rows) > 1 else rows[0]
            pv = jnp.dot(p.astype(jnp.bfloat16), v, preferred_element_type=jnp.float32)
            if fill:
                fill.pop(0)()
            for a in range(mr // R):
                ia = roff // R + a
                pa = p[a * R:(a + 1) * R, :]
                ps = pa[:, 0:128]
                for b in range(1, clen // 128):
                    ps = ps + pa[:, b * 128:(b + 1) * 128]
                lv[ia] = ps if lv[ia] is None else lv[ia] + ps
                t = pv[a * R:(a + 1) * R, :]
                acc[ia] = t if acc[ia] is None else acc[ia] + t
        for a in range(nsub):
            l = jnp.sum(lv[a], axis=-1, keepdims=True)
            o = acc[a] * (1.0 / l)
            ok = (l >= L_LO) & (l <= L_HI) & (jnp.abs(o) <= 3.0e38)
            nb = jnp.where(ok, 0, 1).astype(jnp.int32)
            for i in range(R // 8):
                bad = jnp.maximum(bad, nb[i * 8:(i + 1) * 8, :])
            o_ref[pl.ds(r0 + a * R, R), :] = o.astype(o_ref.dtype)
    return bad


def _attn_exact(q_ref, k_ref, v_ref, o_ref, bq=256, bk=256):
    scale = D ** -0.5

    def q_body(qi, carry):
        rs = pl.ds(pl.multiple_of(qi * bq, bq), bq)
        q = q_ref[rs, :]

        def k_body(kj, st):
            m, l, acc = st
            ks = pl.ds(pl.multiple_of(kj * bk, bk), bk)
            s = lax.dot_general(q, k_ref[ks, :], NT, preferred_element_type=jnp.float32) * scale
            row = lax.broadcasted_iota(jnp.int32, (bq, bk), 0) + qi * bq
            col = lax.broadcasted_iota(jnp.int32, (bq, bk), 1) + kj * bk
            s = jnp.where(col <= row, s, -1e9)
            m_new = jnp.maximum(m, jnp.max(s, axis=-1, keepdims=True))
            p = jnp.exp(s - m_new)
            alpha = jnp.exp(m - m_new)
            l = alpha * l + jnp.sum(p, axis=-1, keepdims=True)
            acc = alpha * acc + jnp.dot(p.astype(jnp.bfloat16), v_ref[ks, :],
                                        preferred_element_type=jnp.float32)
            return m_new, l, acc

        init = (jnp.full((bq, 1), -jnp.inf, jnp.float32), jnp.zeros((bq, 1), jnp.float32),
                jnp.zeros((bq, D), jnp.float32))
        m, l, acc = lax.fori_loop(0, SEQ // bk, k_body, init)
        o_ref[rs, :] = (acc / l).astype(o_ref.dtype)
        return carry

    lax.fori_loop(0, SEQ // bq, q_body, 0)


def _unpack2(u):
    return (pltpu.bitcast(u << 16, jnp.float32), pltpu.bitcast(u & jnp.uint32(HI16), jnp.float32))


def _b_stage1(j, xb, dfw_ref, fm_ref, tv):
    ridx = 127 - lax.broadcasted_iota(jnp.int32, (N1, 128), 1)
    q0, q1r, q2, q3r = [], [], [], []
    for t in range(2):
        q0.append(_unpack2(xb[j, :, pl.ds(t * 128, 128)]))
        q1r.append(_unpack2(jnp.take_along_axis(xb[j, :, pl.ds((3 - t) * 128, 128)], ridx, axis=1)))
        q2.append(_unpack2(xb[j, :, pl.ds((4 + t) * 128, 128)]))
        q3r.append(_unpack2(jnp.take_along_axis(xb[j, :, pl.ds((7 - t) * 128, 128)], ridx, axis=1)))
    for e in range(2):
        n2 = 2 * j + e
        ee, eo, oe, oo = [], [], [], []
        for t in range(2):
            x0, r1, x2, r3 = q0[t][e], q1r[t][e], q2[t][e], q3r[t][e]
            a = x0 + r3
            b = x0 - r3
            c = r1 + x2
            dd = r1 - x2
            ee.append((a + c).astype(jnp.bfloat16))
            eo.append((a - c).astype(jnp.bfloat16))
            oe.append((b - dd).astype(jnp.bfloat16))
            oo.append((b + dd).astype(jnp.bfloat16))
        ee, eo, oe, oo = (jnp.concatenate(z, axis=1) for z in (ee, eo, oe, oo))
        ur_e = lax.dot_general(dfw_ref[pl.ds(0, 256), :], ee, NT, preferred_element_type=jnp.float32)
        ur_o = lax.dot_general(dfw_ref[pl.ds(256, 256), :], eo, NT, preferred_element_type=jnp.float32)
        ui_en = lax.dot_general(dfw_ref[pl.ds(512, 272), :], oe, NT, preferred_element_type=jnp.float32)
        ui_o = lax.dot_general(dfw_ref[pl.ds(784, 256), :], oo, NT, preferred_element_type=jnp.float32)
        ur = jnp.concatenate([ur_e, ur_o, jnp.zeros((16, 128), jnp.float32)], axis=0)
        ui = jnp.concatenate([ui_en[:256], ui_o, ui_en[256:]], axis=0)
        u = jnp.concatenate([ur, ui], axis=1).astype(jnp.bfloat16)
        tv[n2, pl.ds(0, UR), :] = jnp.dot(u, fm_ref[n2], preferred_element_type=jnp.float32)


def _b_stage2(g, nyquist, t_s, v_s, wr_v, wi_v):
    for kind in ((0,) if nyquist else (0, 1)):
        r0 = 512 if nyquist else pl.multiple_of(kind * 256 + g * 8, 8)
        xs = [(t_s[n2, pl.ds(r0, 8), pl.ds(0, 128)], t_s[n2, pl.ds(r0, 8), pl.ds(128, 128)])
              for n2 in range(N2)]
        ys = _fft(xs, -1)
        zs = []
        for k2 in range(N2):
            cs = pl.ds(k2 * 128, 128)
            if nyquist:
                wr = jnp.broadcast_to(wr_v[pl.ds(512, 1), cs].astype(jnp.float32), (8, 128))
                wi = jnp.broadcast_to(wi_v[pl.ds(512, 1), cs].astype(jnp.float32), (8, 128))
            else:
                rows = pl.ds(pl.multiple_of(g * 16, 16), 16)
                wr = _unpack2(pltpu.bitcast(wr_v[rows, cs], jnp.uint32))[kind]
                wi = _unpack2(pltpu.bitcast(wi_v[rows, cs], jnp.uint32))[kind]
            xr, xi = ys[k2]
            zs.append((xr * wr - xi * wi, xr * wi + xi * wr))
        vs = _fft(zs, +1)
        for n2 in range(N2):
            v_s[n2, pl.ds(r0, 8), pl.ds(0, 128)] = vs[n2][0]
            v_s[n2, pl.ds(r0, 8), pl.ds(128, 128)] = vs[n2][1]


def _b_stage3(j, tv, gm_ref, dinv_ref):
    lane = lax.broadcasted_iota(jnp.int32, (N1, 128), 1)
    ridx = 127 - lax.broadcasted_iota(jnp.int32, (N1, 128), 1)
    zr, zi = [], []
    for e in range(2):
        n2 = 2 * j + e
        v = tv[n2].astype(jnp.bfloat16)
        zt = lax.dot_general(gm_ref[n2], v, NT, preferred_element_type=jnp.float32)
        zr.append(zt[:128, :512].astype(jnp.bfloat16))
        zi0 = jnp.where(lane == 0, zt[128:, 512:640], zt[128:, 0:128])
        zi.append(jnp.concatenate([zi0, zt[128:, 128:512]], axis=1).astype(jnp.bfloat16))
    zr = jnp.concatenate(zr, axis=0)
    zi = jnp.concatenate(zi, axis=0)
    pe = jnp.dot(zr[:, :256], dinv_ref[0], preferred_element_type=jnp.float32)
    po = jnp.dot(zr[:, 256:], dinv_ref[1], preferred_element_type=jnp.float32)
    qe = jnp.dot(zi[:, :256], dinv_ref[2], preferred_element_type=jnp.float32)
    qo = jnp.dot(zi[:, 256:], dinv_ref[3], preferred_element_type=jnp.float32)
    ps, pd, qs, qd = pe + po, pe - po, qe + qo, qe - qo
    y0, y1r, y2, y3r = ps - qs, pd + qd, pd - qd, ps + qs

    def pk(y, t):
        return pltpu.pack_elementwise([y[:128, t * 128:(t + 1) * 128], y[128:, t * 128:(t + 1) * 128]],
                                      packed_dtype=jnp.bfloat16)

    outs = [None] * 8
    for t in range(2):
        outs[t] = pk(y0, t)
        outs[3 - t] = jnp.take_along_axis(pk(y1r, t), ridx, axis=1)
        outs[4 + t] = pk(y2, t)
        outs[7 - t] = jnp.take_along_axis(pk(y3r, t), ridx, axis=1)
    return jnp.concatenate(outs, axis=1)


HS = SEQ // 2
ORC = 256
OKG = 4
B1U = 2
B3U = 2
NP = H // 2
B2_IN_HEADS = False
B2_IN_OPROJ = False


def _rhs_ops(b11, b12, b21, b22):
    bf = jnp.bfloat16
    return [lambda: (b11() + b22()).astype(bf), lambda: b11().astype(bf),
            lambda: (b12() - b22()).astype(bf), lambda: (b21() - b11()).astype(bf),
            lambda: b22().astype(bf), lambda: (b11() + b12()).astype(bf),
            lambda: (b21() + b22()).astype(bf)]


def _strassen(lhs, rhs):
    m1, m2, m3, m4, m5, m6, m7 = (jnp.dot(a, b(), preferred_element_type=jnp.float32)
                                  for a, b in zip(lhs, rhs))
    return m1 + m4 - m5 + m7, m3 + m5, m2 + m4, m1 - m2 + m3 + m6


def _kernel(x_hbm, c_hbm, wq_hbm, wk_hbm, wv_hbm, wo_hbm, bx_hbm, wr_hbm, wi_hbm,
            dfw_hbm, dinv_hbm, fm_hbm, gm_hbm, o_hbm,
            x_v, c_v, xs_v, cs_v, wq_b, wk_b, wv_b, wo_v, q_s, k_s, v_s, ctx_s, flags, o_st,
            xb, dfw_v, dinv_v, fm_v, gm_v, wr_v, wi_v, t_s, vv_s, y_st,
            sems, wsem, xsem, fsem, osem, ysem):
    f32, bf16 = jnp.float32, jnp.bfloat16
    wq_u = wq_hbm.bitcast(jnp.uint32)
    wk_u = wk_hbm.bitcast(jnp.uint32)
    wv_u = wv_hbm.bitcast(jnp.uint32)
    bx_u = bx_hbm.bitcast(jnp.uint32)
    o_u = o_hbm.bitcast(jnp.uint32)

    def w_copies(p, slot):
        return [pltpu.make_async_copy(wq_u.at[:, p, :], wq_b.at[slot], wsem.at[slot, 0]),
                pltpu.make_async_copy(wk_u.at[:, p, :], wk_b.at[slot], wsem.at[slot, 1]),
                pltpu.make_async_copy(wv_u.at[:, p, :], wv_b.at[slot], wsem.at[slot, 2])]

    def bx_copy(j):
        return pltpu.make_async_copy(bx_u.at[:, j, :], xb.at[j], xsem.at[j])

    def fm_copy(j):
        return pltpu.make_async_copy(fm_hbm.at[pl.ds(2 * j, 2)], fm_v.at[pl.ds(2 * j, 2)], fsem.at[j])

    def out_copy(r, slot, half):
        n = ORC // N2
        return pltpu.make_async_copy(o_st.at[slot, half],
                                     o_hbm.at[pl.ds(half * (HS // N2) + r * n, n), :, pl.ds(0, M)],
                                     osem.at[slot, half])

    def y_copy(j):
        return pltpu.make_async_copy(y_st.at[j % (2 * B3U)], o_u.at[:, j, pl.ds(M, DB)],
                                     ysem.at[j % (2 * B3U)])

    cp_c = pltpu.make_async_copy(c_hbm, c_v, sems.at[0])
    cp_x = pltpu.make_async_copy(x_hbm, x_v, sems.at[1])
    cp_wr = pltpu.make_async_copy(wr_hbm, wr_v, sems.at[2])
    cp_wi = pltpu.make_async_copy(wi_hbm, wi_v, sems.at[3])
    cp_dfw = pltpu.make_async_copy(dfw_hbm, dfw_v, sems.at[4])
    cp_dinv = pltpu.make_async_copy(dinv_hbm, dinv_v, sems.at[5])
    cp_gm = pltpu.make_async_copy(gm_hbm, gm_v, sems.at[6])
    cp_wo = pltpu.make_async_copy(wo_hbm, wo_v, sems.at[7])

    cp_dfw.start()
    for j in range(N2 // 2):
        bx_copy(j).start()
        fm_copy(j).start()
    cp_c.start()
    cp_x.start()
    for c in w_copies(0, 0):
        c.start()

    vv_s[:, pl.ds(UR, VR - UR), :] = jnp.zeros((N2, VR - UR, 256), f32)
    cp_dfw.wait()
    n1 = N2 // 2 // B1U

    def b1_body(i, carry):
        for u in range(B1U):
            bx_copy(i * B1U + u).wait()
            fm_copy(i * B1U + u).wait()
        for u in range(B1U):
            _b_stage1(i * B1U + u, xb, dfw_v, fm_v, t_s)
        return carry

    lax.fori_loop(0, n1, b1_body, 0)

    def lhs_sums(src, dst, kh):
        def body(r, carry):
            top = pl.ds(pl.multiple_of(r * 128, 128), 128)
            bot = pl.ds(pl.multiple_of(HS + r * 128, 128), 128)
            ops = _strassen_lhs(src[top, pl.ds(0, kh)], src[top, pl.ds(kh, kh)],
                                src[bot, pl.ds(0, kh)], src[bot, pl.ds(kh, kh)])
            for i, o in enumerate((0, 1, 4, 5, 6)):
                dst[i, top, :] = ops[o]
            return carry
        lax.fori_loop(0, HS // 128, body, 0)

    def lhs_load(src, sums, kh):
        top, bot = pl.ds(0, HS), pl.ds(HS, HS)
        return [sums[0], sums[1], src[top, pl.ds(0, kh)], src[bot, pl.ds(kh, kh)],
                sums[2], sums[3], sums[4]]

    cp_c.wait()
    lhs_sums(c_v, cs_v, DC // 2)
    cp_x.wait()
    lhs_sums(x_v, xs_v, M // 2)

    def project_pair(slot):
        top, bot = pl.ds(0, HS), pl.ds(HS, HS)

        def half(buf, r0, n, e):
            return lambda: _unpack2(buf[slot, pl.ds(r0, n), :])[e]

        def kv(e):
            n = DC // 2
            c11, c12, c21, c22 = _strassen(lhs_load(c_v, cs_v, n),
                                           _rhs_ops(half(wk_b, 0, n, e), half(wv_b, 0, n, e),
                                                    half(wk_b, n, n, e), half(wv_b, n, n, e)))
            k_s[e, top, :] = c11.astype(bf16)
            v_s[e, top, :] = c12.astype(bf16)
            k_s[e, bot, :] = c21.astype(bf16)
            v_s[e, bot, :] = c22.astype(bf16)

        kv(0)
        n = M // 2
        c11, c12, c21, c22 = _strassen(lhs_load(x_v, xs_v, n),
                                       _rhs_ops(half(wq_b, 0, n, 0), half(wq_b, 0, n, 1),
                                                half(wq_b, n, n, 0), half(wq_b, n, n, 1)))
        q_s[0, top, :] = (c11 * QSCALE).astype(bf16)
        q_s[1, top, :] = (c12 * QSCALE).astype(bf16)
        q_s[0, bot, :] = (c21 * QSCALE).astype(bf16)
        q_s[1, bot, :] = (c22 * QSCALE).astype(bf16)
        kv(1)

    def pair_body(p, carry):
        slot = p % 2
        for c in w_copies(p, slot):
            c.wait()

        @pl.when(p + 1 < NP)
        def _():
            for c in w_copies(p + 1, 1 - slot):
                c.start()

        @pl.when(p == 1)
        def _():
            cp_wo.start()

        @pl.when(p == 4)
        def _():
            for c in (cp_wr, cp_wi, cp_gm, cp_dinv):
                c.start()

        project_pair(slot)
        fill = []
        if B2_IN_HEADS:
            fill = [functools.partial(_b_stage2, 2 * p + u, False, t_s, vv_s, wr_v, wi_v) for u in range(2)]
        for e in range(2):
            flags[2 * p + e] = _attn_fast(q_s.at[e], k_s.at[e], v_s.at[e], ctx_s.at[2 * p + e], fill)
        return carry

    lax.fori_loop(0, NP, pair_body, 0)

    any_bad = jnp.max(flags[...].reshape(H * 8, 128))

    @pl.when(any_bad > 0)
    def _():
        def redo(h, carry):
            @pl.when(jnp.max(flags[h]) > 0)
            def _():
                p = h // 2
                e = h % 2
                for c in w_copies(p, 0):
                    c.start()
                for c in w_copies(p, 0):
                    c.wait()
                wq = _unpack_head(wq_b.at[0], e)
                wk = _unpack_head(wk_b.at[0], e)
                wv = _unpack_head(wv_b.at[0], e)

                def proj(r, carry):
                    rs = pl.ds(pl.multiple_of(r * 256, 256), 256)
                    cblk = c_v[rs, :]
                    k_s[0, rs, :] = jnp.dot(cblk, wk, preferred_element_type=f32).astype(bf16)
                    v_s[0, rs, :] = jnp.dot(cblk, wv, preferred_element_type=f32).astype(bf16)
                    q_s[0, rs, :] = jnp.dot(x_v[rs, :], wq, preferred_element_type=f32).astype(bf16)
                    return carry
                lax.fori_loop(0, SEQ // 256, proj, 0)
                _attn_exact(q_s.at[0], k_s.at[0], v_s.at[0], ctx_s.at[h])
            return carry
        lax.fori_loop(0, H, redo, 0)

    cp_wr.wait()
    cp_wi.wait()
    cp_wo.wait()
    n_oc = HS // ORC
    gpi = 32 // n_oc

    def oproj_body(r, carry):
        top = pl.ds(pl.multiple_of(r * ORC, ORC), ORC)
        bot = pl.ds(pl.multiple_of(HS + r * ORC, ORC), ORC)
        ng = NP // OKG
        ms = [None] * 7
        for g in range(ng):
            def blk(rows, h0):
                return jnp.concatenate([ctx_s[h0 + g * OKG + i, rows, :] for i in range(OKG)], axis=1)

            def wblk(h0, c0):
                return lambda: wo_v[pl.ds(h0 + g * OKG, OKG), :, pl.ds(c0, M // 2)].reshape(
                    OKG * D, M // 2).astype(f32)
            lhs = _strassen_lhs(blk(top, 0), blk(top, NP), blk(bot, 0), blk(bot, NP))
            rhs = _rhs_ops(wblk(0, 0), wblk(0, M // 2), wblk(NP, 0), wblk(NP, M // 2))
            for i in range(7):
                t = jnp.dot(lhs[i], rhs[i](), preferred_element_type=f32)
                ms[i] = t if ms[i] is None else ms[i] + t
            if B2_IN_OPROJ:
                for u in range(gpi // ng):
                    _b_stage2(r * gpi + g * (gpi // ng) + u, False, t_s, vv_s, wr_v, wi_v)
        m1, m2, m3, m4, m5, m6, m7 = ms
        slot = r % 2

        @pl.when(r >= 2)
        def _():
            for half in range(2):
                out_copy(r - 2, slot, half).wait()

        n = ORC // N2
        for half, (cl, cr) in enumerate(((m1 + m4 - m5 + m7, m3 + m5), (m2 + m4, m1 - m2 + m3 + m6))):
            o_st[slot, half, :, :, pl.ds(0, M // 2)] = cl.astype(bf16).reshape(n, N2, M // 2)
            o_st[slot, half, :, :, pl.ds(M // 2, M // 2)] = cr.astype(bf16).reshape(n, N2, M // 2)
        for half in range(2):
            out_copy(r, slot, half).start()
        return carry

    lax.fori_loop(0, n_oc, oproj_body, 0)

    if not (B2_IN_OPROJ or B2_IN_HEADS):
        def b2_body(g, carry):
            _b_stage2(g, False, t_s, vv_s, wr_v, wi_v)
            return carry
        lax.fori_loop(0, 32, b2_body, 0)
    _b_stage2(0, True, t_s, vv_s, wr_v, wi_v)
    cp_gm.wait()
    cp_dinv.wait()
    n3 = N2 // 2 // B3U

    def b3_body(i, carry):
        ys = [_b_stage3(i * B3U + u, vv_s, gm_v, dinv_v) for u in range(B3U)]

        @pl.when(i >= 2)
        def _():
            for u in range(B3U):
                y_copy((i - 2) * B3U + u).wait()

        for u in range(B3U):
            y_st[(i * B3U + u) % (2 * B3U)] = ys[u]
        for u in range(B3U):
            y_copy(i * B3U + u).start()
        return carry

    lax.fori_loop(0, n3, b3_body, 0)
    for r in (n_oc - 2, n_oc - 1):
        for half in range(2):
            out_copy(r, r % 2, half).wait()
    for j in range((n3 - 2) * B3U, n3 * B3U):
        y_copy(j).wait()


@jax.jit
def pallas_concat_heads__compressed_kv_cla__spectral_gfnet__prompt_kernel(
    A_x: jax.Array,
    A_c_kv: jax.Array,
    A_w_q: jax.Array,
    A_w_uk: jax.Array,
    A_w_uv: jax.Array,
    A_w_o: jax.Array,
    B_x: jax.Array,
    B_w_r: jax.Array,
    B_w_i: jax.Array,
):
    dfw, dinv, fm, gm = _dft_consts()
    hbm = pl.BlockSpec(memory_space=pltpu.HBM)
    bf16, f32, u32 = jnp.bfloat16, jnp.float32, jnp.uint32
    scratch = [
        pltpu.VMEM((SEQ, M), bf16), pltpu.VMEM((SEQ, DC), bf16),
        pltpu.VMEM((5, HS, M // 2), bf16), pltpu.VMEM((5, HS, DC // 2), bf16),
        pltpu.VMEM((2, M, D), u32), pltpu.VMEM((2, DC, D), u32), pltpu.VMEM((2, DC, D), u32),
        pltpu.VMEM((H, D, M), bf16),
        pltpu.VMEM((2, SEQ, D), bf16), pltpu.VMEM((2, SEQ, D), bf16), pltpu.VMEM((2, SEQ, D), bf16),
        pltpu.VMEM((H, SEQ, D), bf16),
        pltpu.VMEM((H, 8, 128), jnp.int32),
        pltpu.VMEM((2, 2, ORC // N2, N2, M), bf16),
        pltpu.VMEM((N2 // 2, N1, DB), u32),
        pltpu.VMEM(dfw.shape, bf16), pltpu.VMEM(dinv.shape, bf16),
        pltpu.VMEM(fm.shape, bf16), pltpu.VMEM(gm.shape, bf16),
        pltpu.VMEM((DF, SB), bf16), pltpu.VMEM((DF, SB), bf16),
        pltpu.VMEM((N2, UR, 256), f32), pltpu.VMEM((N2, VR, 256), f32),
        pltpu.VMEM((2 * B3U, N1, DB), u32),
        pltpu.SemaphoreType.DMA((8,)), pltpu.SemaphoreType.DMA((2, 3)),
        pltpu.SemaphoreType.DMA((N2 // 2,)), pltpu.SemaphoreType.DMA((N2 // 2,)),
        pltpu.SemaphoreType.DMA((2, 2)), pltpu.SemaphoreType.DMA((2 * B3U,)),
    ]
    out = pl.pallas_call(
        _kernel,
        out_shape=jax.ShapeDtypeStruct((N1, N2, M + DB), bf16),
        in_specs=[hbm] * 13,
        out_specs=hbm,
        scratch_shapes=scratch,
        compiler_params=pltpu.CompilerParams(vmem_limit_bytes=126 * 2 ** 20),
    )(A_x.reshape(SEQ, M), A_c_kv.reshape(SEQ, DC), A_w_q, A_w_uk, A_w_uv, A_w_o,
      B_x.reshape(N1, N2, DB), B_w_r.T, B_w_i.T, dfw, dinv, fm, gm)
    return out.reshape(1, SEQ, M + DB)
```

```python
import functools
import math

import jax
import jax.numpy as jnp
import jax.experimental.pallas as pl
import jax.experimental.pallas.tpu as pltpu
import ml_dtypes
import numpy as np
from jax import lax

SEQ = 2048
D = 128
H = 32
M = 1024
DC = 512
SB = 2048
DB = 1024
DF = DB // 2 + 1
N1 = 128
N2 = 16
UR = 528
VR = 640
NT = (((1,), (1,)), ((), ()))
QSCALE = (D ** -0.5) * math.log2(math.e)
L_LO = 2.0 ** -30
L_HI = 2.0 ** 30
HI16 = 0xFFFF0000


@functools.lru_cache(maxsize=None)
def _dft_consts():
    th = 2 * np.pi / DB
    d = np.arange(256, dtype=np.float64) + 0.5
    m = np.arange(256, dtype=np.float64)
    fe, fo = 2 * m, 2 * m + 1
    sny = np.zeros((16, 256))
    sny[0] = -np.sin(th * 512 * d)
    dfw = np.concatenate([np.cos(th * np.outer(fe, d)), np.cos(th * np.outer(fo, d)),
                          -np.sin(th * np.outer(fe, d)), sny, -np.sin(th * np.outer(fo, d))], 0)
    cfe = np.full(256, 2.0 / DB)
    cfe[0] = 1.0 / DB
    cfo = np.full(256, 2.0 / DB)
    gse = cfe[:, None] * np.sin(th * np.outer(fe, d))
    gse[0] = (1.0 / DB) * np.sin(th * 512 * d)
    dinv = np.stack([cfe[:, None] * np.cos(th * np.outer(fe, d)),
                     cfo[:, None] * np.cos(th * np.outer(fo, d)),
                     gse, cfo[:, None] * np.sin(th * np.outer(fo, d))], 0)
    n2 = np.arange(N2)[:, None, None]
    n1 = np.arange(N1)[None, :, None]
    k1 = np.arange(N1)[None, None, :]
    ang = -2 * np.pi * k1 * (N2 * n1 + n2) / SB
    fr, fi = np.cos(ang), np.sin(ang)
    fm = np.concatenate([np.concatenate([fr, fi], 2), np.concatenate([-fi, fr], 2)], 1)
    gr, gi = fr / SB, -fi / SB
    gm = np.concatenate([np.concatenate([gr, -gi], 2), np.concatenate([gi, gr], 2)], 1)
    bf = ml_dtypes.bfloat16
    return tuple(np.asarray(a, dtype=np.float32).astype(bf) for a in (dfw, dinv, fm, gm))


def _cmul_const(xr, xi, ang):
    c, s = math.cos(ang), math.sin(ang)
    eps = 1e-9
    if abs(s) < eps:
        return (xr, xi) if c > 0 else (-xr, -xi)
    if abs(c) < eps:
        return (-xi, xr) if s > 0 else (xi, -xr)
    if abs(abs(c) - abs(s)) < eps:
        if c * s > 0:
            return (xr - xi) * c, (xr + xi) * c
        return (xr + xi) * c, (xi - xr) * c
    return xr * c - xi * s, xr * s + xi * c


def _fft(xs, sign):
    n = len(xs)
    if n == 1:
        return xs
    if n == 2:
        (ar, ai), (br, bi) = xs
        return [(ar + br, ai + bi), (ar - br, ai - bi)]
    if n == 4:
        (ar, ai), (br, bi), (cr, ci), (dr, di) = xs
        t0r, t0i = ar + cr, ai + ci
        t1r, t1i = ar - cr, ai - ci
        t2r, t2i = br + dr, bi + di
        t3r, t3i = br - dr, bi - di
        if sign > 0:
            return [(t0r + t2r, t0i + t2i), (t1r - t3i, t1i + t3r),
                    (t0r - t2r, t0i - t2i), (t1r + t3i, t1i - t3r)]
        return [(t0r + t2r, t0i + t2i), (t1r + t3i, t1i - t3r),
                (t0r - t2r, t0i - t2i), (t1r - t3i, t1i + t3r)]
    ev = _fft(xs[0::2], sign)
    od = _fft(xs[1::2], sign)
    out = [None] * n
    for k in range(n // 2):
        er, ei = ev[k]
        if k * 4 == n:
            o_r, o_i = od[k]
            if sign > 0:
                out[k] = (er - o_i, ei + o_r)
                out[k + n // 2] = (er + o_i, ei - o_r)
            else:
                out[k] = (er + o_i, ei - o_r)
                out[k + n // 2] = (er - o_i, ei + o_r)
        else:
            tr, ti = _cmul_const(od[k][0], od[k][1], sign * 2 * math.pi * k / n)
            out[k] = (er + tr, ei + ti)
            out[k + n // 2] = (er - tr, ei - ti)
    return out


def _unpack_head(wbuf, e):
    sh = (16 * (1 - e)).astype(jnp.uint32)
    w = pltpu.bitcast((wbuf[...] << sh) & jnp.uint32(HI16), jnp.float32)
    return w.astype(jnp.bfloat16)


def _strassen_rhs(b11, b12, b21, b22):
    bf = jnp.bfloat16
    return [(b11 + b22).astype(bf), b11.astype(bf), (b12 - b22).astype(bf), (b21 - b11).astype(bf),
            b22.astype(bf), (b11 + b12).astype(bf), (b21 + b22).astype(bf)]


def _strassen_lhs(a11, a12, a21, a22):
    bf = jnp.bfloat16
    f11, f12, f21, f22 = (a.astype(jnp.float32) for a in (a11, a12, a21, a22))
    return [(f11 + f22).astype(bf), (f21 + f22).astype(bf), a11, a22,
            (f11 + f12).astype(bf), (f21 - f11).astype(bf), (f12 - f22).astype(bf)]


def _strassen_out(lhs, rhs):
    m1, m2, m3, m4, m5, m6, m7 = (jnp.dot(a, b, preferred_element_type=jnp.float32)
                                  for a, b in zip(lhs, rhs))
    return m1 + m4 - m5 + m7, m3 + m5, m2 + m4, m1 - m2 + m3 + m6


def _attn_plan(qi, bq, bk, stair):
    r0 = qi * bq
    steps = []
    c = 0
    while c + bk <= r0:
        steps.append((0, c, bk))
        c += bk
    if c < r0:
        steps.append((0, c, r0 - c))
    for t in range(bq // stair):
        steps.append((t * stair, r0 + t * stair, stair))
    return steps


def _attn_fast(q_ref, k_ref, v_ref, o_ref, fill=None, bq=512, bk=512, stair=128):
    R = 128
    row = lax.broadcasted_iota(jnp.int32, (R, 128), 0)
    col = lax.broadcasted_iota(jnp.int32, (R, 128), 1)
    tri = col <= row
    bad = jnp.zeros((8, 128), jnp.int32)
    for qi in range(SEQ // bq):
        r0 = qi * bq
        nsub = bq // R
        acc = [None] * nsub
        lv = [None] * nsub
        for (roff, c0, clen) in _attn_plan(qi, bq, bk, stair):
            mr = bq - roff
            q = q_ref[pl.ds(r0 + roff, mr), :]
            k = k_ref[pl.ds(c0, clen), :]
            v = v_ref[pl.ds(c0, clen), :]
            s = lax.dot_general(q, k, NT, preferred_element_type=jnp.float32)
            p = jnp.exp2(s)
            if c0 + clen - 1 > r0 + roff:
                rows = []
                for a in range(mr // R):
                    ra = r0 + roff + a * R
                    cols = []
                    for b in range(clen // 128):
                        cb = c0 + b * 128
                        t = p[a * R:(a + 1) * R, b * 128:(b + 1) * 128]
                        if cb == ra:
                            t = jnp.where(tri, t, 0.0)
                        elif cb > ra:
                            t = jnp.zeros_like(t)
                        cols.append(t)
                    rows.append(jnp.concatenate(cols, axis=1) if len(cols) > 1 else cols[0])
                p = jnp.concatenate(rows, axis=0) if len(rows) > 1 else rows[0]
            pv = jnp.dot(p.astype(jnp.bfloat16), v, preferred_element_type=jnp.float32)
            if fill:
                fill.pop(0)()
            for a in range(mr // R):
                ia = roff // R + a
                pa = p[a * R:(a + 1) * R, :]
                ps = pa[:, 0:128]
                for b in range(1, clen // 128):
                    ps = ps + pa[:, b * 128:(b + 1) * 128]
                lv[ia] = ps if lv[ia] is None else lv[ia] + ps
                t = pv[a * R:(a + 1) * R, :]
                acc[ia] = t if acc[ia] is None else acc[ia] + t
        for a in range(nsub):
            l = jnp.sum(lv[a], axis=-1, keepdims=True)
            o = acc[a] * (1.0 / l)
            ok = (l >= L_LO) & (l <= L_HI) & (jnp.abs(o) <= 3.0e38)
            nb = jnp.where(ok, 0, 1).astype(jnp.int32)
            for i in range(R // 8):
                bad = jnp.maximum(bad, nb[i * 8:(i + 1) * 8, :])
            o_ref[pl.ds(r0 + a * R, R), :] = o.astype(o_ref.dtype)
    return bad


def _attn_exact(q_ref, k_ref, v_ref, o_ref, bq=256, bk=256):
    scale = D ** -0.5

    def q_body(qi, carry):
        rs = pl.ds(pl.multiple_of(qi * bq, bq), bq)
        q = q_ref[rs, :]

        def k_body(kj, st):
            m, l, acc = st
            ks = pl.ds(pl.multiple_of(kj * bk, bk), bk)
            s = lax.dot_general(q, k_ref[ks, :], NT, preferred_element_type=jnp.float32) * scale
            row = lax.broadcasted_iota(jnp.int32, (bq, bk), 0) + qi * bq
            col = lax.broadcasted_iota(jnp.int32, (bq, bk), 1) + kj * bk
            s = jnp.where(col <= row, s, -1e9)
            m_new = jnp.maximum(m, jnp.max(s, axis=-1, keepdims=True))
            p = jnp.exp(s - m_new)
            alpha = jnp.exp(m - m_new)
            l = alpha * l + jnp.sum(p, axis=-1, keepdims=True)
            acc = alpha * acc + jnp.dot(p.astype(jnp.bfloat16), v_ref[ks, :],
                                        preferred_element_type=jnp.float32)
            return m_new, l, acc

        init = (jnp.full((bq, 1), -jnp.inf, jnp.float32), jnp.zeros((bq, 1), jnp.float32),
                jnp.zeros((bq, D), jnp.float32))
        m, l, acc = lax.fori_loop(0, SEQ // bk, k_body, init)
        o_ref[rs, :] = (acc / l).astype(o_ref.dtype)
        return carry

    lax.fori_loop(0, SEQ // bq, q_body, 0)


def _unpack2(u):
    return (pltpu.bitcast(u << 16, jnp.float32), pltpu.bitcast(u & jnp.uint32(HI16), jnp.float32))


def _b_stage1(j, xb, dfw_ref, fm_ref, tv):
    ridx = 127 - lax.broadcasted_iota(jnp.int32, (N1, 128), 1)
    q0, q1r, q2, q3r = [], [], [], []
    for t in range(2):
        q0.append(_unpack2(xb[j, :, pl.ds(t * 128, 128)]))
        q1r.append(_unpack2(jnp.take_along_axis(xb[j, :, pl.ds((3 - t) * 128, 128)], ridx, axis=1)))
        q2.append(_unpack2(xb[j, :, pl.ds((4 + t) * 128, 128)]))
        q3r.append(_unpack2(jnp.take_along_axis(xb[j, :, pl.ds((7 - t) * 128, 128)], ridx, axis=1)))
    for e in range(2):
        n2 = 2 * j + e
        ee, eo, oe, oo = [], [], [], []
        for t in range(2):
            x0, r1, x2, r3 = q0[t][e], q1r[t][e], q2[t][e], q3r[t][e]
            a = x0 + r3
            b = x0 - r3
            c = r1 + x2
            dd = r1 - x2
            ee.append((a + c).astype(jnp.bfloat16))
            eo.append((a - c).astype(jnp.bfloat16))
            oe.append((b - dd).astype(jnp.bfloat16))
            oo.append((b + dd).astype(jnp.bfloat16))
        ee, eo, oe, oo = (jnp.concatenate(z, axis=1) for z in (ee, eo, oe, oo))
        ur_e = lax.dot_general(dfw_ref[pl.ds(0, 256), :], ee, NT, preferred_element_type=jnp.float32)
        ur_o = lax.dot_general(dfw_ref[pl.ds(256, 256), :], eo, NT, preferred_element_type=jnp.float32)
        ui_en = lax.dot_general(dfw_ref[pl.ds(512, 272), :], oe, NT, preferred_element_type=jnp.float32)
        ui_o = lax.dot_general(dfw_ref[pl.ds(784, 256), :], oo, NT, preferred_element_type=jnp.float32)
        ur = jnp.concatenate([ur_e, ur_o, jnp.zeros((16, 128), jnp.float32)], axis=0)
        ui = jnp.concatenate([ui_en[:256], ui_o, ui_en[256:]], axis=0)
        u = jnp.concatenate([ur, ui], axis=1).astype(jnp.bfloat16)
        tv[n2, pl.ds(0, UR), :] = jnp.dot(u, fm_ref[n2], preferred_element_type=jnp.float32)


def _b_stage2(g, nyquist, t_s, v_s, wr_v, wi_v):
    for kind in ((0,) if nyquist else (0, 1)):
        r0 = 512 if nyquist else (kind * 256 + g * 8 if isinstance(g, int) else pl.multiple_of(kind * 256 + g * 8, 8))
        xs = [(t_s[n2, pl.ds(r0, 8), pl.ds(0, 128)], t_s[n2, pl.ds(r0, 8), pl.ds(128, 128)])
              for n2 in range(N2)]
        ys = _fft(xs, -1)
        zs = []
        for k2 in range(N2):
            cs = pl.ds(k2 * 128, 128)
            if nyquist:
                wr = jnp.broadcast_to(wr_v[pl.ds(512, 1), cs].astype(jnp.float32), (8, 128))
                wi = jnp.broadcast_to(wi_v[pl.ds(512, 1), cs].astype(jnp.float32), (8, 128))
            else:
                rows = pl.ds(g * 16 if isinstance(g, int) else pl.multiple_of(g * 16, 16), 16)
                wr = _unpack2(pltpu.bitcast(wr_v[rows, cs], jnp.uint32))[kind]
                wi = _unpack2(pltpu.bitcast(wi_v[rows, cs], jnp.uint32))[kind]
            xr, xi = ys[k2]
            zs.append((xr * wr - xi * wi, xr * wi + xi * wr))
        vs = _fft(zs, +1)
        for n2 in range(N2):
            v_s[n2, pl.ds(r0, 8), pl.ds(0, 128)] = vs[n2][0]
            v_s[n2, pl.ds(r0, 8), pl.ds(128, 128)] = vs[n2][1]


def _b_stage3(j, tv, gm_ref, dinv_ref):
    lane = lax.broadcasted_iota(jnp.int32, (N1, 128), 1)
    ridx = 127 - lax.broadcasted_iota(jnp.int32, (N1, 128), 1)
    zr, zi = [], []
    for e in range(2):
        n2 = 2 * j + e
        v = tv[n2].astype(jnp.bfloat16)
        zt = lax.dot_general(gm_ref[n2], v, NT, preferred_element_type=jnp.float32)
        zr.append(zt[:128, :512].astype(jnp.bfloat16))
        zi0 = jnp.where(lane == 0, zt[128:, 512:640], zt[128:, 0:128])
        zi.append(jnp.concatenate([zi0, zt[128:, 128:512]], axis=1).astype(jnp.bfloat16))
    zr = jnp.concatenate(zr, axis=0)
    zi = jnp.concatenate(zi, axis=0)
    pe = jnp.dot(zr[:, :256], dinv_ref[0], preferred_element_type=jnp.float32)
    po = jnp.dot(zr[:, 256:], dinv_ref[1], preferred_element_type=jnp.float32)
    qe = jnp.dot(zi[:, :256], dinv_ref[2], preferred_element_type=jnp.float32)
    qo = jnp.dot(zi[:, 256:], dinv_ref[3], preferred_element_type=jnp.float32)
    ps, pd, qs, qd = pe + po, pe - po, qe + qo, qe - qo
    y0, y1r, y2, y3r = ps - qs, pd + qd, pd - qd, ps + qs

    def pk(y, t):
        return pltpu.pack_elementwise([y[:128, t * 128:(t + 1) * 128], y[128:, t * 128:(t + 1) * 128]],
                                      packed_dtype=jnp.bfloat16)

    outs = [None] * 8
    for t in range(2):
        outs[t] = pk(y0, t)
        outs[3 - t] = jnp.take_along_axis(pk(y1r, t), ridx, axis=1)
        outs[4 + t] = pk(y2, t)
        outs[7 - t] = jnp.take_along_axis(pk(y3r, t), ridx, axis=1)
    return jnp.concatenate(outs, axis=1)


HS = SEQ // 2
ORC = 512
OKG = 2
B1U = 2
B3U = 2
NP = H // 2

SRC = 32
B2_IN_HEADS = False
B2_IN_OPROJ = True


def _rhs_ops(b11, b12, b21, b22):
    bf = jnp.bfloat16
    return [lambda: (b11() + b22()).astype(bf), lambda: b11().astype(bf),
            lambda: (b12() - b22()).astype(bf), lambda: (b21() - b11()).astype(bf),
            lambda: b22().astype(bf), lambda: (b11() + b12()).astype(bf),
            lambda: (b21() + b22()).astype(bf)]


def _strassen(lhs, rhs):
    m1, m2, m3, m4, m5, m6, m7 = (jnp.dot(a, b(), preferred_element_type=jnp.float32)
                                  for a, b in zip(lhs, rhs))
    return m1 + m4 - m5 + m7, m3 + m5, m2 + m4, m1 - m2 + m3 + m6


def _kernel(x_hbm, c_hbm, wq_hbm, wk_hbm, wv_hbm, wo_hbm, bx_hbm, wr_hbm, wi_hbm,
            dfw_hbm, dinv_hbm, fm_hbm, gm_hbm, o_hbm,
            x_v, c_v, xs_v, cs_v, wq_b, wk_b, wv_b, wo_v, q_s, k_s, v_s, ctx_s, flags, o_st,
            xb, dfw_v, dinv_v, fm_v, gm_v, wr_v, wi_v, t_s, vv_s, y_st,
            sems, wsem, xsem, fsem, osem, ysem):
    f32, bf16 = jnp.float32, jnp.bfloat16
    wq_u = wq_hbm.bitcast(jnp.uint32)
    wk_u = wk_hbm.bitcast(jnp.uint32)
    wv_u = wv_hbm.bitcast(jnp.uint32)
    bx_u = bx_hbm.bitcast(jnp.uint32)
    o_u = o_hbm.bitcast(jnp.uint32)

    def w_copies(p, slot):
        return [pltpu.make_async_copy(wq_u.at[:, p, :], wq_b.at[slot], wsem.at[slot, 0]),
                pltpu.make_async_copy(wk_u.at[:, p, :], wk_b.at[slot], wsem.at[slot, 1]),
                pltpu.make_async_copy(wv_u.at[:, p, :], wv_b.at[slot], wsem.at[slot, 2])]

    def bx_copy(j):
        return pltpu.make_async_copy(bx_u.at[:, j, :], xb.at[j], xsem.at[j])

    def fm_copy(j):
        return pltpu.make_async_copy(fm_hbm.at[pl.ds(2 * j, 2)], fm_v.at[pl.ds(2 * j, 2)], fsem.at[j])

    def out_copy(r, slot, half):
        n = ORC // N2
        return pltpu.make_async_copy(o_st.at[slot, half],
                                     o_hbm.at[pl.ds(half * (HS // N2) + r * n, n), :, pl.ds(0, M)],
                                     osem.at[slot, half])

    def y_copy(j):
        return pltpu.make_async_copy(y_st.at[j % (2 * B3U)], o_u.at[:, j, pl.ds(M, DB)],
                                     ysem.at[j % (2 * B3U)])

    cp_c = pltpu.make_async_copy(c_hbm, c_v, sems.at[0])
    cp_x = pltpu.make_async_copy(x_hbm, x_v, sems.at[1])
    cp_wr = pltpu.make_async_copy(wr_hbm, wr_v, sems.at[2])
    cp_wi = pltpu.make_async_copy(wi_hbm, wi_v, sems.at[3])
    cp_dfw = pltpu.make_async_copy(dfw_hbm, dfw_v, sems.at[4])
    cp_dinv = pltpu.make_async_copy(dinv_hbm, dinv_v, sems.at[5])
    cp_gm = pltpu.make_async_copy(gm_hbm, gm_v, sems.at[6])
    cp_wo = pltpu.make_async_copy(wo_hbm, wo_v, sems.at[7])

    cp_dfw.start()
    for j in range(N2 // 2):
        bx_copy(j).start()
        fm_copy(j).start()

    vv_s[:, pl.ds(UR, VR - UR), :] = jnp.zeros((N2, VR - UR, 256), f32)
    cp_dfw.wait()
    n1 = N2 // 2 // B1U

    def b1_body(i, carry):
        for u in range(B1U):
            bx_copy(i * B1U + u).wait()
            fm_copy(i * B1U + u).wait()

        @pl.when(i == 1)
        def _():
            cp_c.start()
            cp_x.start()
            for c in w_copies(0, 0):
                c.start()

        for u in range(B1U):
            _b_stage1(i * B1U + u, xb, dfw_v, fm_v, t_s)
        return carry

    lax.fori_loop(0, n1, b1_body, 0)

    def lhs_sums(src, dst, kh):
        def body(r, carry):
            top = pl.ds(pl.multiple_of(r * SRC, SRC), SRC)
            bot = pl.ds(pl.multiple_of(HS + r * SRC, SRC), SRC)
            ops = _strassen_lhs(src[top, pl.ds(0, kh)], src[top, pl.ds(kh, kh)],
                                src[bot, pl.ds(0, kh)], src[bot, pl.ds(kh, kh)])
            for i, o in enumerate((0, 1, 4, 5, 6)):
                dst[i, top, :] = ops[o]
            return carry
        lax.fori_loop(0, HS // SRC, body, 0)

    def lhs_load(src, sums, kh):
        top, bot = pl.ds(0, HS), pl.ds(HS, HS)
        return [sums[0], sums[1], src[top, pl.ds(0, kh)], src[bot, pl.ds(kh, kh)],
                sums[2], sums[3], sums[4]]

    cp_c.wait()
    lhs_sums(c_v, cs_v, DC // 2)
    cp_x.wait()
    lhs_sums(x_v, xs_v, M // 2)

    def project_pair(slot):
        top, bot = pl.ds(0, HS), pl.ds(HS, HS)

        def half(buf, r0, n, e):
            return lambda: _unpack2(buf[slot, pl.ds(r0, n), :])[e]

        def kv(e):
            n = DC // 2
            c11, c12, c21, c22 = _strassen(lhs_load(c_v, cs_v, n),
                                           _rhs_ops(half(wk_b, 0, n, e), half(wv_b, 0, n, e),
                                                    half(wk_b, n, n, e), half(wv_b, n, n, e)))
            k_s[e, top, :] = c11.astype(bf16)
            v_s[e, top, :] = c12.astype(bf16)
            k_s[e, bot, :] = c21.astype(bf16)
            v_s[e, bot, :] = c22.astype(bf16)

        kv(0)
        n = M // 2
        c11, c12, c21, c22 = _strassen(lhs_load(x_v, xs_v, n),
                                       _rhs_ops(half(wq_b, 0, n, 0), half(wq_b, 0, n, 1),
                                                half(wq_b, n, n, 0), half(wq_b, n, n, 1)))
        q_s[0, top, :] = (c11 * QSCALE).astype(bf16)
        q_s[1, top, :] = (c12 * QSCALE).astype(bf16)
        q_s[0, bot, :] = (c21 * QSCALE).astype(bf16)
        q_s[1, bot, :] = (c22 * QSCALE).astype(bf16)
        kv(1)

    def pair_body(p, carry):
        slot = p % 2
        for c in w_copies(p, slot):
            c.wait()

        @pl.when(p + 1 < NP)
        def _():
            for c in w_copies(p + 1, 1 - slot):
                c.start()

        @pl.when(p == 1)
        def _():
            cp_wo.start()

        @pl.when(p == 4)
        def _():
            for c in (cp_wr, cp_wi, cp_gm, cp_dinv):
                c.start()

        project_pair(slot)
        fill = []
        if B2_IN_HEADS:
            fill = [functools.partial(_b_stage2, 2 * p + u, False, t_s, vv_s, wr_v, wi_v) for u in range(2)]
        for e in range(2):
            flags[2 * p + e] = _attn_fast(q_s.at[e], k_s.at[e], v_s.at[e], ctx_s.at[2 * p + e], fill)
        return carry

    lax.fori_loop(0, NP, pair_body, 0)

    any_bad = jnp.max(flags[...].reshape(H * 8, 128))

    @pl.when(any_bad > 0)
    def _():
        def redo(h, carry):
            @pl.when(jnp.max(flags[h]) > 0)
            def _():
                p = h // 2
                e = h % 2
                for c in w_copies(p, 0):
                    c.start()
                for c in w_copies(p, 0):
                    c.wait()
                wq = _unpack_head(wq_b.at[0], e)
                wk = _unpack_head(wk_b.at[0], e)
                wv = _unpack_head(wv_b.at[0], e)

                def proj(r, carry):
                    rs = pl.ds(pl.multiple_of(r * 256, 256), 256)
                    cblk = c_v[rs, :]
                    k_s[0, rs, :] = jnp.dot(cblk, wk, preferred_element_type=f32).astype(bf16)
                    v_s[0, rs, :] = jnp.dot(cblk, wv, preferred_element_type=f32).astype(bf16)
                    q_s[0, rs, :] = jnp.dot(x_v[rs, :], wq, preferred_element_type=f32).astype(bf16)
                    return carry
                lax.fori_loop(0, SEQ // 256, proj, 0)
                _attn_exact(q_s.at[0], k_s.at[0], v_s.at[0], ctx_s.at[h])
            return carry
        lax.fori_loop(0, H, redo, 0)

    cp_wr.wait()
    cp_wi.wait()
    cp_wo.wait()
    n_oc = HS // ORC
    gpi = 32 // n_oc

    def oproj_body(r):
        top = pl.ds(r * ORC, ORC)
        bot = pl.ds(HS + r * ORC, ORC)
        ng = NP // OKG
        ms = [None] * 7
        for g in range(ng):
            def blk(rows, h0):
                return jnp.concatenate([ctx_s[h0 + g * OKG + i, rows, :] for i in range(OKG)], axis=1)

            def wblk(h0, c0):
                return lambda: wo_v[pl.ds(h0 + g * OKG, OKG), :, pl.ds(c0, M // 2)].reshape(
                    OKG * D, M // 2).astype(f32)
            lhs = _strassen_lhs(blk(top, 0), blk(top, NP), blk(bot, 0), blk(bot, NP))
            rhs = _rhs_ops(wblk(0, 0), wblk(0, M // 2), wblk(NP, 0), wblk(NP, M // 2))
            for i in range(7):
                t = jnp.dot(lhs[i], rhs[i](), preferred_element_type=f32)
                ms[i] = t if ms[i] is None else ms[i] + t
                if B2_IN_OPROJ and i in (1, 4):
                    idx = g * 2 + (i == 4)
                    for u in range(gpi // (2 * ng)):
                        _b_stage2(r * gpi + idx * (gpi // (2 * ng)) + u, False, t_s, vv_s, wr_v, wi_v)
        m1, m2, m3, m4, m5, m6, m7 = ms
        slot = r
        n = ORC // N2
        for half, (cl, cr) in enumerate(((m1 + m4 - m5 + m7, m3 + m5), (m2 + m4, m1 - m2 + m3 + m6))):
            o_st[slot, half, :, :, pl.ds(0, M // 2)] = cl.astype(bf16).reshape(n, N2, M // 2)
            o_st[slot, half, :, :, pl.ds(M // 2, M // 2)] = cr.astype(bf16).reshape(n, N2, M // 2)
        for half in range(2):
            out_copy(r, slot, half).start()

    for r in range(n_oc):
        oproj_body(r)

    if not (B2_IN_OPROJ or B2_IN_HEADS):
        def b2_body(g, carry):
            _b_stage2(g, False, t_s, vv_s, wr_v, wi_v)
            return carry
        lax.fori_loop(0, 32, b2_body, 0)
    _b_stage2(0, True, t_s, vv_s, wr_v, wi_v)
    cp_gm.wait()
    cp_dinv.wait()
    n3 = N2 // 2 // B3U

    def b3_body(i, carry):
        ys = [_b_stage3(i * B3U + u, vv_s, gm_v, dinv_v) for u in range(B3U)]

        @pl.when(i >= 2)
        def _():
            for u in range(B3U):
                y_copy((i - 2) * B3U + u).wait()

        for u in range(B3U):
            y_st[(i * B3U + u) % (2 * B3U)] = ys[u]
        for u in range(B3U):
            y_copy(i * B3U + u).start()
        return carry

    lax.fori_loop(0, n3, b3_body, 0)
    for r in (n_oc - 2, n_oc - 1):
        for half in range(2):
            out_copy(r, r % 2, half).wait()
    for j in range((n3 - 2) * B3U, n3 * B3U):
        y_copy(j).wait()


@jax.jit
def pallas_concat_heads__compressed_kv_cla__spectral_gfnet__prompt_kernel(
    A_x: jax.Array,
    A_c_kv: jax.Array,
    A_w_q: jax.Array,
    A_w_uk: jax.Array,
    A_w_uv: jax.Array,
    A_w_o: jax.Array,
    B_x: jax.Array,
    B_w_r: jax.Array,
    B_w_i: jax.Array,
):
    dfw, dinv, fm, gm = _dft_consts()
    hbm = pl.BlockSpec(memory_space=pltpu.HBM)
    bf16, f32, u32 = jnp.bfloat16, jnp.float32, jnp.uint32
    scratch = [
        pltpu.VMEM((SEQ, M), bf16), pltpu.VMEM((SEQ, DC), bf16),
        pltpu.VMEM((5, HS, M // 2), bf16), pltpu.VMEM((5, HS, DC // 2), bf16),
        pltpu.VMEM((2, M, D), u32), pltpu.VMEM((2, DC, D), u32), pltpu.VMEM((2, DC, D), u32),
        pltpu.VMEM((H, D, M), bf16),
        pltpu.VMEM((2, SEQ, D), bf16), pltpu.VMEM((2, SEQ, D), bf16), pltpu.VMEM((2, SEQ, D), bf16),
        pltpu.VMEM((H, SEQ, D), bf16),
        pltpu.VMEM((H, 8, 128), jnp.int32),
        pltpu.VMEM((2, 2, ORC // N2, N2, M), bf16),
        pltpu.VMEM((N2 // 2, N1, DB), u32),
        pltpu.VMEM(dfw.shape, bf16), pltpu.VMEM(dinv.shape, bf16),
        pltpu.VMEM(fm.shape, bf16), pltpu.VMEM(gm.shape, bf16),
        pltpu.VMEM((DF, SB), bf16), pltpu.VMEM((DF, SB), bf16),
        pltpu.VMEM((N2, UR, 256), f32), pltpu.VMEM((N2, VR, 256), f32),
        pltpu.VMEM((2 * B3U, N1, DB), u32),
        pltpu.SemaphoreType.DMA((8,)), pltpu.SemaphoreType.DMA((2, 3)),
        pltpu.SemaphoreType.DMA((N2 // 2,)), pltpu.SemaphoreType.DMA((N2 // 2,)),
        pltpu.SemaphoreType.DMA((2, 2)), pltpu.SemaphoreType.DMA((2 * B3U,)),
    ]
    out = pl.pallas_call(
        _kernel,
        out_shape=jax.ShapeDtypeStruct((N1, N2, M + DB), bf16),
        in_specs=[hbm] * 13,
        out_specs=hbm,
        scratch_shapes=scratch,
        compiler_params=pltpu.CompilerParams(vmem_limit_bytes=126 * 2 ** 20),
    )(A_x.reshape(SEQ, M), A_c_kv.reshape(SEQ, DC), A_w_q, A_w_uk, A_w_uv, A_w_o,
      B_x.reshape(N1, N2, DB), B_w_r.T, B_w_i.T, dfw, dinv, fm, gm)
    return out.reshape(1, SEQ, M + DB)
```

```python
import functools
import math

import jax
import jax.numpy as jnp
import jax.experimental.pallas as pl
import jax.experimental.pallas.tpu as pltpu
import ml_dtypes
import numpy as np
from jax import lax

SEQ = 2048
D = 128
H = 32
M = 1024
DC = 512
SB = 2048
DB = 1024
DF = DB // 2 + 1
N1 = 128
N2 = 16
UR = 528
VR = 512
NT = (((1,), (1,)), ((), ()))
QSCALE = (D ** -0.5) * math.log2(math.e)
L_LO = 2.0 ** -30
L_HI = 2.0 ** 30
HI16 = 0xFFFF0000

BQ = BK = 512
DIAG_FIRST = True


@functools.lru_cache(maxsize=None)
def _dft_consts():
    th = 2 * np.pi / DB
    d = np.arange(256, dtype=np.float64) + 0.5
    m = np.arange(256, dtype=np.float64)
    fe, fo = 2 * m, 2 * m + 1
    sny = np.zeros((16, 256))
    sny[0] = -np.sin(th * 512 * d)
    dfw = np.concatenate([np.cos(th * np.outer(fe, d)), np.cos(th * np.outer(fo, d)),
                          -np.sin(th * np.outer(fe, d)), sny, -np.sin(th * np.outer(fo, d))], 0)
    cfe = np.full(256, 2.0 / DB)
    cfe[0] = 1.0 / DB
    cfo = np.full(256, 2.0 / DB)
    gse = cfe[:, None] * np.sin(th * np.outer(fe, d))
    gse[0] = (1.0 / DB) * np.sin(th * 512 * d)
    dinv = np.stack([cfe[:, None] * np.cos(th * np.outer(fe, d)),
                     cfo[:, None] * np.cos(th * np.outer(fo, d)),
                     gse, cfo[:, None] * np.sin(th * np.outer(fo, d))], 0)
    n1 = np.arange(N1)[:, None]
    k1 = np.arange(N1)[None, :]
    base = np.stack([np.cos(2 * np.pi * n1 * k1 / N1), -np.sin(2 * np.pi * n1 * k1 / N1)], 0)
    n2 = np.arange(N2)[:, None]
    tw = np.stack([np.cos(2 * np.pi * n2 * k1 / SB), -np.sin(2 * np.pi * n2 * k1 / SB)], 0)
    tw = np.repeat(tw[:, :, None, :], 8, axis=2)
    bf = ml_dtypes.bfloat16
    return (np.asarray(dfw, dtype=np.float32).astype(bf), np.asarray(dinv, dtype=np.float32).astype(bf),
            base.astype(np.float32), tw.astype(np.float32))


def _cmul_const(xr, xi, ang):
    c, s = math.cos(ang), math.sin(ang)
    eps = 1e-9
    if abs(s) < eps:
        return (xr, xi) if c > 0 else (-xr, -xi)
    if abs(c) < eps:
        return (-xi, xr) if s > 0 else (xi, -xr)
    if abs(abs(c) - abs(s)) < eps:
        if c * s > 0:
            return (xr - xi) * c, (xr + xi) * c
        return (xr + xi) * c, (xi - xr) * c
    return xr * c - xi * s, xr * s + xi * c


def _fft(xs, sign):
    n = len(xs)
    if n == 1:
        return xs
    if n == 2:
        (ar, ai), (br, bi) = xs
        return [(ar + br, ai + bi), (ar - br, ai - bi)]
    if n == 4:
        (ar, ai), (br, bi), (cr, ci), (dr, di) = xs
        t0r, t0i = ar + cr, ai + ci
        t1r, t1i = ar - cr, ai - ci
        t2r, t2i = br + dr, bi + di
        t3r, t3i = br - dr, bi - di
        if sign > 0:
            return [(t0r + t2r, t0i + t2i), (t1r - t3i, t1i + t3r),
                    (t0r - t2r, t0i - t2i), (t1r + t3i, t1i - t3r)]
        return [(t0r + t2r, t0i + t2i), (t1r + t3i, t1i - t3r),
                (t0r - t2r, t0i - t2i), (t1r - t3i, t1i + t3r)]
    ev = _fft(xs[0::2], sign)
    od = _fft(xs[1::2], sign)
    out = [None] * n
    for k in range(n // 2):
        er, ei = ev[k]
        if k * 4 == n:
            o_r, o_i = od[k]
            if sign > 0:
                out[k] = (er - o_i, ei + o_r)
                out[k + n // 2] = (er + o_i, ei - o_r)
            else:
                out[k] = (er + o_i, ei - o_r)
                out[k + n // 2] = (er - o_i, ei + o_r)
        else:
            tr, ti = _cmul_const(od[k][0], od[k][1], sign * 2 * math.pi * k / n)
            out[k] = (er + tr, ei + ti)
            out[k + n // 2] = (er - tr, ei - ti)
    return out


def _unpack_head(wbuf, e):
    sh = (16 * (1 - e)).astype(jnp.uint32)
    w = pltpu.bitcast((wbuf[...] << sh) & jnp.uint32(HI16), jnp.float32)
    return w.astype(jnp.bfloat16)


def _strassen_rhs(b11, b12, b21, b22):
    bf = jnp.bfloat16
    return [(b11 + b22).astype(bf), b11.astype(bf), (b12 - b22).astype(bf), (b21 - b11).astype(bf),
            b22.astype(bf), (b11 + b12).astype(bf), (b21 + b22).astype(bf)]


def _strassen_lhs(a11, a12, a21, a22):
    bf = jnp.bfloat16
    f11, f12, f21, f22 = (a.astype(jnp.float32) for a in (a11, a12, a21, a22))
    return [(f11 + f22).astype(bf), (f21 + f22).astype(bf), a11, a22,
            (f11 + f12).astype(bf), (f21 - f11).astype(bf), (f12 - f22).astype(bf)]


def _strassen_out(lhs, rhs):
    m1, m2, m3, m4, m5, m6, m7 = (jnp.dot(a, b, preferred_element_type=jnp.float32)
                                  for a, b in zip(lhs, rhs))
    return m1 + m4 - m5 + m7, m3 + m5, m2 + m4, m1 - m2 + m3 + m6


def _attn_plan(qi, bq, bk, stair):
    r0 = qi * bq
    steps = []
    c = 0
    while c + bk <= r0:
        steps.append((0, c, bk))
        c += bk
    if c < r0:
        steps.append((0, c, r0 - c))
    diag = [(t * stair, r0 + t * stair, stair) for t in range(bq // stair)]
    return diag + steps if DIAG_FIRST else steps + diag


def _attn_fast(q_ref, k_ref, v_ref, o_ref, bq=BQ, bk=BK, stair=128):
    R = 128
    row = lax.broadcasted_iota(jnp.int32, (R, 128), 0)
    col = lax.broadcasted_iota(jnp.int32, (R, 128), 1)
    tri = col <= row
    bad = jnp.zeros((8, 128), jnp.int32)
    for qi in range(SEQ // bq):
        r0 = qi * bq
        nsub = bq // R
        acc = [None] * nsub
        lv = [None] * nsub
        for (roff, c0, clen) in _attn_plan(qi, bq, bk, stair):
            mr = bq - roff
            q = q_ref[pl.ds(r0 + roff, mr), :]
            k = k_ref[pl.ds(c0, clen), :]
            v = v_ref[pl.ds(c0, clen), :]
            s = lax.dot_general(q, k, NT, preferred_element_type=jnp.float32)
            p = jnp.exp2(s)
            if c0 + clen - 1 > r0 + roff:
                rows = []
                for a in range(mr // R):
                    ra = r0 + roff + a * R
                    cols = []
                    for b in range(clen // 128):
                        cb = c0 + b * 128
                        t = p[a * R:(a + 1) * R, b * 128:(b + 1) * 128]
                        if cb == ra:
                            t = jnp.where(tri, t, 0.0)
                        elif cb > ra:
                            t = jnp.zeros_like(t)
                        cols.append(t)
                    rows.append(jnp.concatenate(cols, axis=1) if len(cols) > 1 else cols[0])
                p = jnp.concatenate(rows, axis=0) if len(rows) > 1 else rows[0]
            pv = jnp.dot(p.astype(jnp.bfloat16), v, preferred_element_type=jnp.float32)
            for a in range(mr // R):
                ia = roff // R + a
                pa = p[a * R:(a + 1) * R, :]
                ps = pa[:, 0:128]
                for b in range(1, clen // 128):
                    ps = ps + pa[:, b * 128:(b + 1) * 128]
                lv[ia] = ps if lv[ia] is None else lv[ia] + ps
                t = pv[a * R:(a + 1) * R, :]
                acc[ia] = t if acc[ia] is None else acc[ia] + t
        for a in range(nsub):
            l = jnp.sum(lv[a], axis=-1, keepdims=True)
            o = acc[a] * (1.0 / l)
            ok = (l >= L_LO) & (l <= L_HI) & (jnp.abs(o) <= 3.0e38)
            nb = jnp.where(ok, 0, 1).astype(jnp.int32)
            for i in range(R // 8):
                bad = jnp.maximum(bad, nb[i * 8:(i + 1) * 8, :])
            o_ref[pl.ds(r0 + a * R, R), :] = o.astype(o_ref.dtype)
    return bad


def _attn_exact(q_ref, k_ref, v_ref, o_ref, bq=256, bk=256):
    scale = D ** -0.5

    def q_body(qi, carry):
        rs = pl.ds(pl.multiple_of(qi * bq, bq), bq)
        q = q_ref[rs, :]

        def k_body(kj, st):
            m, l, acc = st
            ks = pl.ds(pl.multiple_of(kj * bk, bk), bk)
            s = lax.dot_general(q, k_ref[ks, :], NT, preferred_element_type=jnp.float32) * scale
            row = lax.broadcasted_iota(jnp.int32, (bq, bk), 0) + qi * bq
            col = lax.broadcasted_iota(jnp.int32, (bq, bk), 1) + kj * bk
            s = jnp.where(col <= row, s, -1e9)
            m_new = jnp.maximum(m, jnp.max(s, axis=-1, keepdims=True))
            p = jnp.exp(s - m_new)
            alpha = jnp.exp(m - m_new)
            l = alpha * l + jnp.sum(p, axis=-1, keepdims=True)
            acc = alpha * acc + jnp.dot(p.astype(jnp.bfloat16), v_ref[ks, :],
                                        preferred_element_type=jnp.float32)
            return m_new, l, acc

        init = (jnp.full((bq, 1), -jnp.inf, jnp.float32), jnp.zeros((bq, 1), jnp.float32),
                jnp.zeros((bq, D), jnp.float32))
        m, l, acc = lax.fori_loop(0, SEQ // bk, k_body, init)
        o_ref[rs, :] = (acc / l).astype(o_ref.dtype)
        return carry

    lax.fori_loop(0, SEQ // bq, q_body, 0)


def _unpack2(u):
    return (pltpu.bitcast(u << 16, jnp.float32), pltpu.bitcast(u & jnp.uint32(HI16), jnp.float32))


def _s_matrix(n2, base_ref, tw_ref):
    fr, fi = [], []
    for r in range(N1 // 8):
        br = base_ref[0, pl.ds(r * 8, 8), :]
        bi = base_ref[1, pl.ds(r * 8, 8), :]
        tr = tw_ref[0, n2]
        ti = tw_ref[1, n2]
        fr.append(br * tr - bi * ti)
        fi.append(br * ti + bi * tr)
    return jnp.concatenate(fr, axis=0), jnp.concatenate(fi, axis=0)


def _b_stage1(j, xb, dfw_ref, base_ref, tw_ref, tv):
    bf = jnp.bfloat16
    ridx = 127 - lax.broadcasted_iota(jnp.int32, (N1, 128), 1)
    q0, q1r, q2, q3r = [], [], [], []
    for t in range(2):
        q0.append(_unpack2(xb[j, :, pl.ds(t * 128, 128)]))
        q1r.append(_unpack2(jnp.take_along_axis(xb[j, :, pl.ds((3 - t) * 128, 128)], ridx, axis=1)))
        q2.append(_unpack2(xb[j, :, pl.ds((4 + t) * 128, 128)]))
        q3r.append(_unpack2(jnp.take_along_axis(xb[j, :, pl.ds((7 - t) * 128, 128)], ridx, axis=1)))
    for e in range(2):
        n2 = 2 * j + e
        ee, eo, oe, oo = [], [], [], []
        for t in range(2):
            x0, r1, x2, r3 = q0[t][e], q1r[t][e], q2[t][e], q3r[t][e]
            a = x0 + r3
            b = x0 - r3
            c = r1 + x2
            dd = r1 - x2
            ee.append((a + c).astype(jnp.bfloat16))
            eo.append((a - c).astype(jnp.bfloat16))
            oe.append((b - dd).astype(jnp.bfloat16))
            oo.append((b + dd).astype(jnp.bfloat16))
        ee, eo, oe, oo = (jnp.concatenate(z, axis=1) for z in (ee, eo, oe, oo))
        ur_e = lax.dot_general(dfw_ref[pl.ds(0, 256), :], ee, NT, preferred_element_type=jnp.float32)
        ur_o = lax.dot_general(dfw_ref[pl.ds(256, 256), :], eo, NT, preferred_element_type=jnp.float32)
        ui_en = lax.dot_general(dfw_ref[pl.ds(512, 272), :], oe, NT, preferred_element_type=jnp.float32)
        ui_o = lax.dot_general(dfw_ref[pl.ds(784, 256), :], oo, NT, preferred_element_type=jnp.float32)
        ur = jnp.concatenate([ur_e, ur_o, jnp.zeros((16, 128), jnp.float32)], axis=0)
        ui = jnp.concatenate([ui_en[:256], ui_o, ui_en[256:]], axis=0)
        fr, fi = _s_matrix(n2, base_ref, tw_ref)
        k1 = jnp.dot(ur.astype(bf), fr.astype(bf), preferred_element_type=jnp.float32)
        k2 = jnp.dot(ui.astype(bf), fi.astype(bf), preferred_element_type=jnp.float32)
        k3 = jnp.dot((ur + ui).astype(bf), (fr + fi).astype(bf), preferred_element_type=jnp.float32)
        tv[n2, pl.ds(0, UR), pl.ds(0, 128)] = k1 - k2
        tv[n2, pl.ds(0, UR), pl.ds(128, 128)] = k3 - k1 - k2


def _b_filtered(r0, t_s, w_of):
    xs = [(t_s[n2, pl.ds(r0, 8), pl.ds(0, 128)], t_s[n2, pl.ds(r0, 8), pl.ds(128, 128)])
          for n2 in range(N2)]
    zs = []
    for k2, (xr, xi) in enumerate(_fft(xs, -1)):
        wr, wi = w_of(pl.ds(k2 * 128, 128))
        zs.append((xr * wr - xi * wi, xr * wi + xi * wr))
    return zs


def _b_stage2(g, t_s, v_s, wr_v, wi_v):
    for kind in (0, 1):
        r0 = kind * 256 + g * 8

        def w_of(cs):
            return tuple(_unpack2(pltpu.bitcast(w[pl.ds(g * 16, 16), cs], jnp.uint32))[kind]
                         for w in (wr_v, wi_v))
        zs = _b_filtered(r0, t_s, w_of)
        if g == 0 and kind == 0:
            def w_ny(cs):
                return tuple(jnp.broadcast_to(w[pl.ds(512, 1), cs].astype(jnp.float32), (8, 128))
                             for w in (wr_v, wi_v))
            ns = _b_filtered(512, t_s, w_ny)
            lane = lax.broadcasted_iota(jnp.int32, (8, 128), 1)
            row = lax.broadcasted_iota(jnp.int32, (8, 128), 0)
            idx = (128 - lane) % 128
            da = [z[0] - n[0] for z, n in zip(zs, ns)]
            db = [n[1] - z[1] for z, n in zip(zs, ns)]

            def rev(x, k2):
                return jnp.where(lane == 0, x[(N2 - k2) % N2],
                                 jnp.take_along_axis(x[N2 - 1 - k2], idx, axis=1))
            zs = [(jnp.where(row == 0, 0.5 * (z[0] + n[0] + rev(da, k2)), z[0]),
                   jnp.where(row == 0, 0.5 * (z[1] + n[1] + rev(db, k2)), z[1]))
                  for k2, (z, n) in enumerate(zip(zs, ns))]
        vs = _fft(zs, +1)
        for n2 in range(N2):
            v_s[n2, pl.ds(r0, 8), pl.ds(0, 128)] = vs[n2][0]
            v_s[n2, pl.ds(r0, 8), pl.ds(128, 128)] = vs[n2][1]


def _b_stage3(j, tv, base_ref, tw_ref, dinv_ref):
    bf = jnp.bfloat16
    ridx = 127 - lax.broadcasted_iota(jnp.int32, (N1, 128), 1)
    zr, zi = [], []
    for e in range(2):
        n2 = 2 * j + e
        vr = tv[n2, :, pl.ds(0, 128)]
        vi = tv[n2, :, pl.ds(128, 128)]
        fr, fi = _s_matrix(n2, base_ref, tw_ref)
        gr, gi = fr * (1.0 / SB), fi * (-1.0 / SB)
        k1 = lax.dot_general(gr.astype(bf), vr.astype(bf), NT, preferred_element_type=jnp.float32)
        k2 = lax.dot_general(gi.astype(bf), vi.astype(bf), NT, preferred_element_type=jnp.float32)
        k3 = lax.dot_general((gr + gi).astype(bf), (vr + vi).astype(bf), NT,
                             preferred_element_type=jnp.float32)
        zr.append((k1 - k2).astype(bf))
        zi.append((k3 - k1 - k2).astype(bf))
    zr = jnp.concatenate(zr, axis=0)
    zi = jnp.concatenate(zi, axis=0)
    pe = jnp.dot(zr[:, :256], dinv_ref[0], preferred_element_type=jnp.float32)
    po = jnp.dot(zr[:, 256:], dinv_ref[1], preferred_element_type=jnp.float32)
    qe = jnp.dot(zi[:, :256], dinv_ref[2], preferred_element_type=jnp.float32)
    qo = jnp.dot(zi[:, 256:], dinv_ref[3], preferred_element_type=jnp.float32)
    ps, pd, qs, qd = pe + po, pe - po, qe + qo, qe - qo
    y0, y1r, y2, y3r = ps - qs, pd + qd, pd - qd, ps + qs

    def pk(y, t):
        return pltpu.pack_elementwise([y[:128, t * 128:(t + 1) * 128], y[128:, t * 128:(t + 1) * 128]],
                                      packed_dtype=jnp.bfloat16)

    outs = [None] * 8
    for t in range(2):
        outs[t] = pk(y0, t)
        outs[3 - t] = jnp.take_along_axis(pk(y1r, t), ridx, axis=1)
        outs[4 + t] = pk(y2, t)
        outs[7 - t] = jnp.take_along_axis(pk(y3r, t), ridx, axis=1)
    return jnp.concatenate(outs, axis=1)


HS = SEQ // 2
ORC = 512
OKG = 2
B1U = 2
B3U = 2
NP = H // 2

SRC = 32


def _rhs_ops(b11, b12, b21, b22):
    bf = jnp.bfloat16
    return [lambda: (b11() + b22()).astype(bf), lambda: b11().astype(bf),
            lambda: (b12() - b22()).astype(bf), lambda: (b21() - b11()).astype(bf),
            lambda: b22().astype(bf), lambda: (b11() + b12()).astype(bf),
            lambda: (b21() + b22()).astype(bf)]


def _strassen(lhs, rhs):
    m1, m2, m3, m4, m5, m6, m7 = (jnp.dot(a, b(), preferred_element_type=jnp.float32)
                                  for a, b in zip(lhs, rhs))
    return m1 + m4 - m5 + m7, m3 + m5, m2 + m4, m1 - m2 + m3 + m6


def _kernel(x_hbm, c_hbm, wq_hbm, wk_hbm, wv_hbm, wo_hbm, bx_hbm, wr_hbm, wi_hbm,
            dfw_hbm, dinv_hbm, base_hbm, tw_hbm, o_hbm,
            x_v, c_v, xs_v, cs_v, wq_b, wk_b, wv_b, wo_v, q_s, k_s, v_s, ctx_s, flags, o_st,
            xb, dfw_v, dinv_v, base_v, tw_v, wr_v, wi_v, t_s, vv_s, y_st,
            sems, wsem, xsem, osem, ysem):
    f32, bf16 = jnp.float32, jnp.bfloat16
    wq_u = wq_hbm.bitcast(jnp.uint32)
    wk_u = wk_hbm.bitcast(jnp.uint32)
    wv_u = wv_hbm.bitcast(jnp.uint32)
    bx_u = bx_hbm.bitcast(jnp.uint32)
    o_u = o_hbm.bitcast(jnp.uint32)

    def w_copies(p, slot):
        return [pltpu.make_async_copy(wq_u.at[:, p, :], wq_b.at[slot], wsem.at[slot, 0]),
                pltpu.make_async_copy(wk_u.at[:, p, :], wk_b.at[slot], wsem.at[slot, 1]),
                pltpu.make_async_copy(wv_u.at[:, p, :], wv_b.at[slot], wsem.at[slot, 2])]

    def bx_copy(j):
        return pltpu.make_async_copy(bx_u.at[:, j, :], xb.at[j], xsem.at[j])

    def out_copy(r, slot, half):
        n = ORC // N2
        return pltpu.make_async_copy(o_st.at[slot, half],
                                     o_hbm.at[pl.ds(half * (HS // N2) + r * n, n), :, pl.ds(0, M)],
                                     osem.at[slot, half])

    def y_copy(j):
        return pltpu.make_async_copy(y_st.at[j % (2 * B3U)], o_u.at[:, j, pl.ds(M, DB)],
                                     ysem.at[j % (2 * B3U)])

    cp_c = pltpu.make_async_copy(c_hbm, c_v, sems.at[0])
    cp_x = pltpu.make_async_copy(x_hbm, x_v, sems.at[1])
    cp_wr = pltpu.make_async_copy(wr_hbm, wr_v, sems.at[2])
    cp_wi = pltpu.make_async_copy(wi_hbm, wi_v, sems.at[3])
    cp_dfw = pltpu.make_async_copy(dfw_hbm, dfw_v, sems.at[4])
    cp_dinv = pltpu.make_async_copy(dinv_hbm, dinv_v, sems.at[5])
    cp_base = pltpu.make_async_copy(base_hbm, base_v, sems.at[6])
    cp_tw = pltpu.make_async_copy(tw_hbm, tw_v, sems.at[8])
    cp_wo = pltpu.make_async_copy(wo_hbm, wo_v, sems.at[7])

    for c in (cp_dfw, cp_base, cp_tw):
        c.start()
    for j in range(N2 // 2):
        bx_copy(j).start()

    for c in (cp_dfw, cp_base, cp_tw):
        c.wait()
    n1 = N2 // 2 // B1U

    def b1_body(i, carry):
        for u in range(B1U):
            bx_copy(i * B1U + u).wait()

        @pl.when(i == 0)
        def _():
            cp_c.start()
            cp_x.start()
            for c in w_copies(0, 0):
                c.start()

        for u in range(B1U):
            _b_stage1(i * B1U + u, xb, dfw_v, base_v, tw_v, t_s)
        return carry

    lax.fori_loop(0, n1, b1_body, 0)

    def lhs_sums(src, dst, kh):
        def body(r, carry):
            top = pl.ds(pl.multiple_of(r * SRC, SRC), SRC)
            bot = pl.ds(pl.multiple_of(HS + r * SRC, SRC), SRC)
            ops = _strassen_lhs(src[top, pl.ds(0, kh)], src[top, pl.ds(kh, kh)],
                                src[bot, pl.ds(0, kh)], src[bot, pl.ds(kh, kh)])
            for i, o in enumerate((0, 1, 4, 5, 6)):
                dst[i, top, :] = ops[o]
            return carry
        lax.fori_loop(0, HS // SRC, body, 0)

    def lhs_load(src, sums, kh):
        top, bot = pl.ds(0, HS), pl.ds(HS, HS)
        return [sums[0], sums[1], src[top, pl.ds(0, kh)], src[bot, pl.ds(kh, kh)],
                sums[2], sums[3], sums[4]]

    cp_c.wait()
    lhs_sums(c_v, cs_v, DC // 2)
    cp_x.wait()
    lhs_sums(x_v, xs_v, M // 2)

    def project_pair(slot):
        top, bot = pl.ds(0, HS), pl.ds(HS, HS)

        def half(buf, r0, n, e):
            return lambda: _unpack2(buf[slot, pl.ds(r0, n), :])[e]

        def kv(e):
            n = DC // 2
            c11, c12, c21, c22 = _strassen(lhs_load(c_v, cs_v, n),
                                           _rhs_ops(half(wk_b, 0, n, e), half(wv_b, 0, n, e),
                                                    half(wk_b, n, n, e), half(wv_b, n, n, e)))
            k_s[e, top, :] = c11.astype(bf16)
            v_s[e, top, :] = c12.astype(bf16)
            k_s[e, bot, :] = c21.astype(bf16)
            v_s[e, bot, :] = c22.astype(bf16)

        kv(0)
        n = M // 2
        c11, c12, c21, c22 = _strassen(lhs_load(x_v, xs_v, n),
                                       _rhs_ops(half(wq_b, 0, n, 0), half(wq_b, 0, n, 1),
                                                half(wq_b, n, n, 0), half(wq_b, n, n, 1)))
        q_s[0, top, :] = (c11 * QSCALE).astype(bf16)
        q_s[1, top, :] = (c12 * QSCALE).astype(bf16)
        q_s[0, bot, :] = (c21 * QSCALE).astype(bf16)
        q_s[1, bot, :] = (c22 * QSCALE).astype(bf16)
        kv(1)

    def pair_body(p, carry):
        slot = p % 2
        for c in w_copies(p, slot):
            c.wait()

        @pl.when(p + 1 < NP)
        def _():
            for c in w_copies(p + 1, 1 - slot):
                c.start()

        @pl.when(p == 1)
        def _():
            cp_wo.start()

        @pl.when(p == 4)
        def _():
            for c in (cp_wr, cp_wi, cp_dinv):
                c.start()

        project_pair(slot)
        for e in range(2):
            flags[2 * p + e] = _attn_fast(q_s.at[e], k_s.at[e], v_s.at[e], ctx_s.at[2 * p + e])
        return carry

    lax.fori_loop(0, NP, pair_body, 0)

    any_bad = jnp.max(flags[...].reshape(H * 8, 128))

    @pl.when(any_bad > 0)
    def _():
        def redo(h, carry):
            @pl.when(jnp.max(flags[h]) > 0)
            def _():
                p = h // 2
                e = h % 2
                for c in w_copies(p, 0):
                    c.start()
                for c in w_copies(p, 0):
                    c.wait()
                wq = _unpack_head(wq_b.at[0], e)
                wk = _unpack_head(wk_b.at[0], e)
                wv = _unpack_head(wv_b.at[0], e)

                def proj(r, carry):
                    rs = pl.ds(pl.multiple_of(r * 256, 256), 256)
                    cblk = c_v[rs, :]
                    k_s[0, rs, :] = jnp.dot(cblk, wk, preferred_element_type=f32).astype(bf16)
                    v_s[0, rs, :] = jnp.dot(cblk, wv, preferred_element_type=f32).astype(bf16)
                    q_s[0, rs, :] = jnp.dot(x_v[rs, :], wq, preferred_element_type=f32).astype(bf16)
                    return carry
                lax.fori_loop(0, SEQ // 256, proj, 0)
                _attn_exact(q_s.at[0], k_s.at[0], v_s.at[0], ctx_s.at[h])
            return carry
        lax.fori_loop(0, H, redo, 0)

    cp_wr.wait()
    cp_wi.wait()
    cp_wo.wait()
    n_oc = HS // ORC
    gpi = 32 // n_oc

    def oproj_body(r):
        top = pl.ds(r * ORC, ORC)
        bot = pl.ds(HS + r * ORC, ORC)
        ng = NP // OKG
        ms = [None] * 7
        for g in range(ng):
            def blk(rows, h0):
                return jnp.concatenate([ctx_s[h0 + g * OKG + i, rows, :] for i in range(OKG)], axis=1)

            def wblk(h0, c0):
                return lambda: wo_v[pl.ds(h0 + g * OKG, OKG), :, pl.ds(c0, M // 2)].reshape(
                    OKG * D, M // 2).astype(f32)
            lhs = _strassen_lhs(blk(top, 0), blk(top, NP), blk(bot, 0), blk(bot, NP))
            rhs = _rhs_ops(wblk(0, 0), wblk(0, M // 2), wblk(NP, 0), wblk(NP, M // 2))
            for i in range(7):
                t = jnp.dot(lhs[i], rhs[i](), preferred_element_type=f32)
                ms[i] = t if ms[i] is None else ms[i] + t
                if i in (1, 4):
                    idx = g * 2 + (i == 4)
                    for u in range(gpi // (2 * ng)):
                        _b_stage2(r * gpi + idx * (gpi // (2 * ng)) + u, t_s, vv_s, wr_v, wi_v)
        m1, m2, m3, m4, m5, m6, m7 = ms
        slot = r
        n = ORC // N2
        for half, (cl, cr) in enumerate(((m1 + m4 - m5 + m7, m3 + m5), (m2 + m4, m1 - m2 + m3 + m6))):
            o_st[slot, half, :, :, pl.ds(0, M // 2)] = cl.astype(bf16).reshape(n, N2, M // 2)
            o_st[slot, half, :, :, pl.ds(M // 2, M // 2)] = cr.astype(bf16).reshape(n, N2, M // 2)
        for half in range(2):
            out_copy(r, slot, half).start()

    for r in range(n_oc):
        oproj_body(r)

    cp_dinv.wait()
    n3 = N2 // 2 // B3U

    def b3_body(i, carry):
        @pl.when(i >= 2)
        def _():
            for u in range(B3U):
                y_copy((i - 2) * B3U + u).wait()

        ys = [_b_stage3(i * B3U + u, vv_s, base_v, tw_v, dinv_v) for u in range(B3U)]
        for u in range(B3U):
            y_st[(i * B3U + u) % (2 * B3U)] = ys[u]
        for u in range(B3U):
            y_copy(i * B3U + u).start()
        return carry

    lax.fori_loop(0, n3, b3_body, 0)
    for r in (n_oc - 2, n_oc - 1):
        for half in range(2):
            out_copy(r, r % 2, half).wait()
    for j in range((n3 - 2) * B3U, n3 * B3U):
        y_copy(j).wait()


@jax.jit
def pallas_concat_heads__compressed_kv_cla__spectral_gfnet__prompt_kernel(
    A_x: jax.Array,
    A_c_kv: jax.Array,
    A_w_q: jax.Array,
    A_w_uk: jax.Array,
    A_w_uv: jax.Array,
    A_w_o: jax.Array,
    B_x: jax.Array,
    B_w_r: jax.Array,
    B_w_i: jax.Array,
):
    dfw, dinv, base, tw = _dft_consts()
    hbm = pl.BlockSpec(memory_space=pltpu.HBM)
    bf16, f32, u32 = jnp.bfloat16, jnp.float32, jnp.uint32
    scratch = [
        pltpu.VMEM((SEQ, M), bf16), pltpu.VMEM((SEQ, DC), bf16),
        pltpu.VMEM((5, HS, M // 2), bf16), pltpu.VMEM((5, HS, DC // 2), bf16),
        pltpu.VMEM((2, M, D), u32), pltpu.VMEM((2, DC, D), u32), pltpu.VMEM((2, DC, D), u32),
        pltpu.VMEM((H, D, M), bf16),
        pltpu.VMEM((2, SEQ, D), bf16), pltpu.VMEM((2, SEQ, D), bf16), pltpu.VMEM((2, SEQ, D), bf16),
        pltpu.VMEM((H, SEQ, D), bf16),
        pltpu.VMEM((H, 8, 128), jnp.int32),
        pltpu.VMEM((2, 2, ORC // N2, N2, M), bf16),
        pltpu.VMEM((N2 // 2, N1, DB), u32),
        pltpu.VMEM(dfw.shape, bf16), pltpu.VMEM(dinv.shape, bf16),
        pltpu.VMEM(base.shape, f32), pltpu.VMEM(tw.shape, f32),
        pltpu.VMEM((DF, SB), bf16), pltpu.VMEM((DF, SB), bf16),
        pltpu.VMEM((N2, UR, 256), f32), pltpu.VMEM((N2, VR, 256), f32),
        pltpu.VMEM((2 * B3U, N1, DB), u32),
        pltpu.SemaphoreType.DMA((9,)), pltpu.SemaphoreType.DMA((2, 3)),
        pltpu.SemaphoreType.DMA((N2 // 2,)),
        pltpu.SemaphoreType.DMA((2, 2)), pltpu.SemaphoreType.DMA((2 * B3U,)),
    ]
    out = pl.pallas_call(
        _kernel,
        out_shape=jax.ShapeDtypeStruct((N1, N2, M + DB), bf16),
        in_specs=[hbm] * 13,
        out_specs=hbm,
        scratch_shapes=scratch,
        compiler_params=pltpu.CompilerParams(vmem_limit_bytes=126 * 2 ** 20),
    )(A_x.reshape(SEQ, M), A_c_kv.reshape(SEQ, DC), A_w_q, A_w_uk, A_w_uv, A_w_o,
      B_x.reshape(N1, N2, DB), B_w_r.T, B_w_i.T, dfw, dinv, base, tw)
    return out.reshape(1, SEQ, M + DB)
```

```python
import functools
import math

import jax
import jax.numpy as jnp
import jax.experimental.pallas as pl
import jax.experimental.pallas.tpu as pltpu
import ml_dtypes
import numpy as np
from jax import lax

SEQ = 2048
D = 128
H = 32
M = 1024
DC = 512
SB = 2048
DB = 1024
DF = DB // 2 + 1
N1 = 128
N2 = 16
UR = 528
VR = 512
NT = (((1,), (1,)), ((), ()))
QSCALE = (D ** -0.5) * math.log2(math.e)
L_LO = 2.0 ** -30
L_HI = 2.0 ** 30
HI16 = 0xFFFF0000
BQ = BK = 512


@functools.lru_cache(maxsize=None)
def _dft_consts():
    th = 2 * np.pi / DB
    d = np.arange(256, dtype=np.float64) + 0.5
    m = np.arange(256, dtype=np.float64)
    fe, fo = 2 * m, 2 * m + 1
    sny = np.zeros((16, 256))
    sny[0] = -np.sin(th * 512 * d)
    dfw = np.concatenate([np.cos(th * np.outer(fe, d)), np.cos(th * np.outer(fo, d)),
                          -np.sin(th * np.outer(fe, d)), sny, -np.sin(th * np.outer(fo, d))], 0)
    cfe = np.full(256, 2.0 / DB)
    cfe[0] = 1.0 / DB
    cfo = np.full(256, 2.0 / DB)
    gse = cfe[:, None] * np.sin(th * np.outer(fe, d))
    gse[0] = (1.0 / DB) * np.sin(th * 512 * d)
    dinv = np.stack([cfe[:, None] * np.cos(th * np.outer(fe, d)),
                     cfo[:, None] * np.cos(th * np.outer(fo, d)),
                     gse, cfo[:, None] * np.sin(th * np.outer(fo, d))], 0)
    n1 = np.arange(N1)[:, None]
    k1 = np.arange(N1)[None, :]
    base = np.stack([np.cos(2 * np.pi * n1 * k1 / N1), -np.sin(2 * np.pi * n1 * k1 / N1)], 0)
    n2 = np.arange(N2)[:, None]
    tw = np.stack([np.cos(2 * np.pi * n2 * k1 / SB), -np.sin(2 * np.pi * n2 * k1 / SB)], 0)
    tw = np.repeat(tw[:, :, None, :], 8, axis=2)
    bf = ml_dtypes.bfloat16
    return (np.asarray(dfw, dtype=np.float32).astype(bf), np.asarray(dinv, dtype=np.float32).astype(bf),
            base.astype(np.float32), tw.astype(np.float32))


def _cmul_const(xr, xi, ang):
    c, s = math.cos(ang), math.sin(ang)
    eps = 1e-9
    if abs(s) < eps:
        return (xr, xi) if c > 0 else (-xr, -xi)
    if abs(c) < eps:
        return (-xi, xr) if s > 0 else (xi, -xr)
    if abs(abs(c) - abs(s)) < eps:
        if c * s > 0:
            return (xr - xi) * c, (xr + xi) * c
        return (xr + xi) * c, (xi - xr) * c
    return xr * c - xi * s, xr * s + xi * c


def _fft(xs, sign):
    n = len(xs)
    if n == 1:
        return xs
    if n == 2:
        (ar, ai), (br, bi) = xs
        return [(ar + br, ai + bi), (ar - br, ai - bi)]
    if n == 4:
        (ar, ai), (br, bi), (cr, ci), (dr, di) = xs
        t0r, t0i = ar + cr, ai + ci
        t1r, t1i = ar - cr, ai - ci
        t2r, t2i = br + dr, bi + di
        t3r, t3i = br - dr, bi - di
        if sign > 0:
            return [(t0r + t2r, t0i + t2i), (t1r - t3i, t1i + t3r),
                    (t0r - t2r, t0i - t2i), (t1r + t3i, t1i - t3r)]
        return [(t0r + t2r, t0i + t2i), (t1r + t3i, t1i - t3r),
                (t0r - t2r, t0i - t2i), (t1r - t3i, t1i + t3r)]
    ev = _fft(xs[0::2], sign)
    od = _fft(xs[1::2], sign)
    out = [None] * n
    for k in range(n // 2):
        er, ei = ev[k]
        if k * 4 == n:
            o_r, o_i = od[k]
            if sign > 0:
                out[k] = (er - o_i, ei + o_r)
                out[k + n // 2] = (er + o_i, ei - o_r)
            else:
                out[k] = (er + o_i, ei - o_r)
                out[k + n // 2] = (er - o_i, ei + o_r)
        else:
            tr, ti = _cmul_const(od[k][0], od[k][1], sign * 2 * math.pi * k / n)
            out[k] = (er + tr, ei + ti)
            out[k + n // 2] = (er - tr, ei - ti)
    return out


def _unpack_head(wbuf, e):
    sh = (16 * (1 - e)).astype(jnp.uint32)
    w = pltpu.bitcast((wbuf[...] << sh) & jnp.uint32(HI16), jnp.float32)
    return w.astype(jnp.bfloat16)


def _strassen_lhs(a11, a12, a21, a22):
    bf = jnp.bfloat16
    f11, f12, f21, f22 = (a.astype(jnp.float32) for a in (a11, a12, a21, a22))
    return [(f11 + f22).astype(bf), (f21 + f22).astype(bf), a11, a22,
            (f11 + f12).astype(bf), (f21 - f11).astype(bf), (f12 - f22).astype(bf)]


def _attn_plan(qi, bq, bk, stair):
    r0 = qi * bq
    steps = []
    c = 0
    while c + bk <= r0:
        steps.append((0, c, bk))
        c += bk
    if c < r0:
        steps.append((0, c, r0 - c))
    diag = [(t * stair, r0 + t * stair, stair) for t in range(bq // stair)]
    return diag + steps


def _attn_fast(q_ref, k_ref, v_ref, o_ref, bq=BQ, bk=BK, stair=128):
    R = 128
    row = lax.broadcasted_iota(jnp.int32, (R, 128), 0)
    col = lax.broadcasted_iota(jnp.int32, (R, 128), 1)
    tri = col <= row
    bad = jnp.zeros((8, 128), jnp.int32)
    for qi in range(SEQ // bq):
        r0 = qi * bq
        nsub = bq // R
        acc = [None] * nsub
        lv = [None] * nsub
        for (roff, c0, clen) in _attn_plan(qi, bq, bk, stair):
            mr = bq - roff
            q = q_ref[pl.ds(r0 + roff, mr), :]
            k = k_ref[pl.ds(c0, clen), :]
            v = v_ref[pl.ds(c0, clen), :]
            s = lax.dot_general(q, k, NT, preferred_element_type=jnp.float32)
            p = jnp.exp2(s)
            if c0 + clen - 1 > r0 + roff:
                rows = []
                for a in range(mr // R):
                    ra = r0 + roff + a * R
                    cols = []
                    for b in range(clen // 128):
                        cb = c0 + b * 128
                        t = p[a * R:(a + 1) * R, b * 128:(b + 1) * 128]
                        if cb == ra:
                            t = jnp.where(tri, t, 0.0)
                        elif cb > ra:
                            t = jnp.zeros_like(t)
                        cols.append(t)
                    rows.append(jnp.concatenate(cols, axis=1) if len(cols) > 1 else cols[0])
                p = jnp.concatenate(rows, axis=0) if len(rows) > 1 else rows[0]
            pv = jnp.dot(p.astype(jnp.bfloat16), v, preferred_element_type=jnp.float32)
            for a in range(mr // R):
                ia = roff // R + a
                pa = p[a * R:(a + 1) * R, :]
                ps = pa[:, 0:128]
                for b in range(1, clen // 128):
                    ps = ps + pa[:, b * 128:(b + 1) * 128]
                lv[ia] = ps if lv[ia] is None else lv[ia] + ps
                t = pv[a * R:(a + 1) * R, :]
                acc[ia] = t if acc[ia] is None else acc[ia] + t
        for a in range(nsub):
            l = jnp.sum(lv[a], axis=-1, keepdims=True)
            o = acc[a] * (1.0 / l)
            ok = (l >= L_LO) & (l <= L_HI) & (jnp.abs(o) <= 3.0e38)
            nb = jnp.where(ok, 0, 1).astype(jnp.int32)
            for i in range(R // 8):
                bad = jnp.maximum(bad, nb[i * 8:(i + 1) * 8, :])
            o_ref[pl.ds(r0 + a * R, R), :] = o.astype(o_ref.dtype)
    return bad


def _attn_exact(q_ref, k_ref, v_ref, o_ref, bq=256, bk=256):
    scale = D ** -0.5

    def q_body(qi, carry):
        rs = pl.ds(pl.multiple_of(qi * bq, bq), bq)
        q = q_ref[rs, :]

        def k_body(kj, st):
            m, l, acc = st
            ks = pl.ds(pl.multiple_of(kj * bk, bk), bk)
            s = lax.dot_general(q, k_ref[ks, :], NT, preferred_element_type=jnp.float32) * scale
            row = lax.broadcasted_iota(jnp.int32, (bq, bk), 0) + qi * bq
            col = lax.broadcasted_iota(jnp.int32, (bq, bk), 1) + kj * bk
            s = jnp.where(col <= row, s, -1e9)
            m_new = jnp.maximum(m, jnp.max(s, axis=-1, keepdims=True))
            p = jnp.exp(s - m_new)
            alpha = jnp.exp(m - m_new)
            l = alpha * l + jnp.sum(p, axis=-1, keepdims=True)
            acc = alpha * acc + jnp.dot(p.astype(jnp.bfloat16), v_ref[ks, :],
                                        preferred_element_type=jnp.float32)
            return m_new, l, acc

        init = (jnp.full((bq, 1), -jnp.inf, jnp.float32), jnp.zeros((bq, 1), jnp.float32),
                jnp.zeros((bq, D), jnp.float32))
        m, l, acc = lax.fori_loop(0, SEQ // bk, k_body, init)
        o_ref[rs, :] = (acc / l).astype(o_ref.dtype)
        return carry

    lax.fori_loop(0, SEQ // bq, q_body, 0)


def _unpack2(u):
    return (pltpu.bitcast(u << 16, jnp.float32), pltpu.bitcast(u & jnp.uint32(HI16), jnp.float32))


def _s_matrix(n2, base_ref, tw_ref):
    fr, fi = [], []
    for r in range(N1 // 8):
        br = base_ref[0, pl.ds(r * 8, 8), :]
        bi = base_ref[1, pl.ds(r * 8, 8), :]
        tr = tw_ref[0, n2]
        ti = tw_ref[1, n2]
        fr.append(br * tr - bi * ti)
        fi.append(br * ti + bi * tr)
    return jnp.concatenate(fr, axis=0), jnp.concatenate(fi, axis=0)


def _b_stage1(j, xb, dfw_ref, base_ref, tw_ref, tv):
    bf = jnp.bfloat16
    ridx = 127 - lax.broadcasted_iota(jnp.int32, (N1, 128), 1)
    q0, q1r, q2, q3r = [], [], [], []
    for t in range(2):
        q0.append(_unpack2(xb[j, :, pl.ds(t * 128, 128)]))
        q1r.append(_unpack2(jnp.take_along_axis(xb[j, :, pl.ds((3 - t) * 128, 128)], ridx, axis=1)))
        q2.append(_unpack2(xb[j, :, pl.ds((4 + t) * 128, 128)]))
        q3r.append(_unpack2(jnp.take_along_axis(xb[j, :, pl.ds((7 - t) * 128, 128)], ridx, axis=1)))
    for e in range(2):
        n2 = 2 * j + e
        ee, eo, oe, oo = [], [], [], []
        for t in range(2):
            x0, r1, x2, r3 = q0[t][e], q1r[t][e], q2[t][e], q3r[t][e]
            a = x0 + r3
            b = x0 - r3
            c = r1 + x2
            dd = r1 - x2
            ee.append((a + c).astype(jnp.bfloat16))
            eo.append((a - c).astype(jnp.bfloat16))
            oe.append((b - dd).astype(jnp.bfloat16))
            oo.append((b + dd).astype(jnp.bfloat16))
        ee, eo, oe, oo = (jnp.concatenate(z, axis=1) for z in (ee, eo, oe, oo))
        ur_e = lax.dot_general(dfw_ref[pl.ds(0, 256), :], ee, NT, preferred_element_type=jnp.float32)
        ur_o = lax.dot_general(dfw_ref[pl.ds(256, 256), :], eo, NT, preferred_element_type=jnp.float32)
        ui_en = lax.dot_general(dfw_ref[pl.ds(512, 272), :], oe, NT, preferred_element_type=jnp.float32)
        ui_o = lax.dot_general(dfw_ref[pl.ds(784, 256), :], oo, NT, preferred_element_type=jnp.float32)
        ur = jnp.concatenate([ur_e, ur_o, jnp.zeros((16, 128), jnp.float32)], axis=0)
        ui = jnp.concatenate([ui_en[:256], ui_o, ui_en[256:]], axis=0)
        fr, fi = _s_matrix(n2, base_ref, tw_ref)
        k1 = jnp.dot(ur.astype(bf), fr.astype(bf), preferred_element_type=jnp.float32)
        k2 = jnp.dot(ui.astype(bf), fi.astype(bf), preferred_element_type=jnp.float32)
        k3 = jnp.dot((ur + ui).astype(bf), (fr + fi).astype(bf), preferred_element_type=jnp.float32)
        tv[n2, pl.ds(0, UR), pl.ds(0, 128)] = k1 - k2
        tv[n2, pl.ds(0, UR), pl.ds(128, 128)] = k3 - k1 - k2


def _b_filtered(r0, t_s, w_of):
    xs = [(t_s[n2, pl.ds(r0, 8), pl.ds(0, 128)], t_s[n2, pl.ds(r0, 8), pl.ds(128, 128)])
          for n2 in range(N2)]
    zs = []
    for k2, (xr, xi) in enumerate(_fft(xs, -1)):
        wr, wi = w_of(pl.ds(k2 * 128, 128))
        zs.append((xr * wr - xi * wi, xr * wi + xi * wr))
    return zs


def _b_stage2(g, t_s, v_s, wr_v, wi_v):
    for kind in (0, 1):
        r0 = kind * 256 + g * 8

        def w_of(cs):
            return tuple(_unpack2(pltpu.bitcast(w[pl.ds(g * 16, 16), cs], jnp.uint32))[kind]
                         for w in (wr_v, wi_v))
        zs = _b_filtered(r0, t_s, w_of)
        if g == 0 and kind == 0:
            def w_ny(cs):
                return tuple(jnp.broadcast_to(w[pl.ds(512, 1), cs].astype(jnp.float32), (8, 128))
                             for w in (wr_v, wi_v))
            ns = _b_filtered(512, t_s, w_ny)
            lane = lax.broadcasted_iota(jnp.int32, (8, 128), 1)
            row = lax.broadcasted_iota(jnp.int32, (8, 128), 0)
            idx = (128 - lane) % 128
            da = [z[0] - n[0] for z, n in zip(zs, ns)]
            db = [n[1] - z[1] for z, n in zip(zs, ns)]

            def rev(x, k2):
                return jnp.where(lane == 0, x[(N2 - k2) % N2],
                                 jnp.take_along_axis(x[N2 - 1 - k2], idx, axis=1))
            zs = [(jnp.where(row == 0, 0.5 * (z[0] + n[0] + rev(da, k2)), z[0]),
                   jnp.where(row == 0, 0.5 * (z[1] + n[1] + rev(db, k2)), z[1]))
                  for k2, (z, n) in enumerate(zip(zs, ns))]
        vs = _fft(zs, +1)
        for n2 in range(N2):
            v_s[n2, pl.ds(r0, 8), pl.ds(0, 128)] = vs[n2][0]
            v_s[n2, pl.ds(r0, 8), pl.ds(128, 128)] = vs[n2][1]


def _b_stage3(j, tv, base_ref, tw_ref, dinv_ref):
    bf = jnp.bfloat16
    ridx = 127 - lax.broadcasted_iota(jnp.int32, (N1, 128), 1)
    zr, zi = [], []
    for e in range(2):
        n2 = 2 * j + e
        vr = tv[n2, :, pl.ds(0, 128)]
        vi = tv[n2, :, pl.ds(128, 128)]
        fr, fi = _s_matrix(n2, base_ref, tw_ref)
        gr, gi = fr * (1.0 / SB), fi * (-1.0 / SB)
        k1 = lax.dot_general(gr.astype(bf), vr.astype(bf), NT, preferred_element_type=jnp.float32)
        k2 = lax.dot_general(gi.astype(bf), vi.astype(bf), NT, preferred_element_type=jnp.float32)
        k3 = lax.dot_general((gr + gi).astype(bf), (vr + vi).astype(bf), NT,
                             preferred_element_type=jnp.float32)
        zr.append((k1 - k2).astype(bf))
        zi.append((k3 - k1 - k2).astype(bf))
    zr = jnp.concatenate(zr, axis=0)
    zi = jnp.concatenate(zi, axis=0)
    pe = jnp.dot(zr[:, :256], dinv_ref[0], preferred_element_type=jnp.float32)
    po = jnp.dot(zr[:, 256:], dinv_ref[1], preferred_element_type=jnp.float32)
    qe = jnp.dot(zi[:, :256], dinv_ref[2], preferred_element_type=jnp.float32)
    qo = jnp.dot(zi[:, 256:], dinv_ref[3], preferred_element_type=jnp.float32)
    ps, pd, qs, qd = pe + po, pe - po, qe + qo, qe - qo
    y0, y1r, y2, y3r = ps - qs, pd + qd, pd - qd, ps + qs

    def pk(y, t):
        return pltpu.pack_elementwise([y[:128, t * 128:(t + 1) * 128], y[128:, t * 128:(t + 1) * 128]],
                                      packed_dtype=jnp.bfloat16)

    outs = [None] * 8
    for t in range(2):
        outs[t] = pk(y0, t)
        outs[3 - t] = jnp.take_along_axis(pk(y1r, t), ridx, axis=1)
        outs[4 + t] = pk(y2, t)
        outs[7 - t] = jnp.take_along_axis(pk(y3r, t), ridx, axis=1)
    return jnp.concatenate(outs, axis=1)


HS = SEQ // 2
ORC = 512
OKG = 2
B1U = 2
B3U = 2
NP = H // 2

SRC = 32


def _rhs_ops(b11, b12, b21, b22):
    bf = jnp.bfloat16
    return [lambda: (b11() + b22()).astype(bf), lambda: b11().astype(bf),
            lambda: (b12() - b22()).astype(bf), lambda: (b21() - b11()).astype(bf),
            lambda: b22().astype(bf), lambda: (b11() + b12()).astype(bf),
            lambda: (b21() + b22()).astype(bf)]


def _strassen(lhs, rhs):
    m1, m2, m3, m4, m5, m6, m7 = (jnp.dot(a, b(), preferred_element_type=jnp.float32)
                                  for a, b in zip(lhs, rhs))
    return m1 + m4 - m5 + m7, m3 + m5, m2 + m4, m1 - m2 + m3 + m6


def _kernel(x_hbm, c_hbm, wq_hbm, wk_hbm, wv_hbm, wo_hbm, bx_hbm, wr_hbm, wi_hbm,
            dfw_hbm, dinv_hbm, base_hbm, tw_hbm, o_hbm,
            x_v, c_v, xs_v, cs_v, wq_b, wk_b, wv_b, wo_v, q_s, k_s, v_s, ctx_s, flags, o_st,
            xb, dfw_v, dinv_v, base_v, tw_v, wr_v, wi_v, t_s, vv_s, y_st,
            sems, wsem, xsem, osem, ysem):
    f32, bf16 = jnp.float32, jnp.bfloat16
    wq_u = wq_hbm.bitcast(jnp.uint32)
    wk_u = wk_hbm.bitcast(jnp.uint32)
    wv_u = wv_hbm.bitcast(jnp.uint32)
    bx_u = bx_hbm.bitcast(jnp.uint32)
    o_u = o_hbm.bitcast(jnp.uint32)

    def w_copies(p, slot):
        return [pltpu.make_async_copy(wq_u.at[:, p, :], wq_b.at[slot], wsem.at[slot, 0]),
                pltpu.make_async_copy(wk_u.at[:, p, :], wk_b.at[slot], wsem.at[slot, 1]),
                pltpu.make_async_copy(wv_u.at[:, p, :], wv_b.at[slot], wsem.at[slot, 2])]

    def bx_copy(j):
        return pltpu.make_async_copy(bx_u.at[:, j, :], xb.at[j], xsem.at[j])

    def out_copy(r, slot, half):
        n = ORC // N2
        return pltpu.make_async_copy(o_st.at[slot, half],
                                     o_hbm.at[pl.ds(half * (HS // N2) + r * n, n), :, pl.ds(0, M)],
                                     osem.at[slot, half])

    def y_copy(j):
        return pltpu.make_async_copy(y_st.at[j % (2 * B3U)], o_u.at[:, j, pl.ds(M, DB)],
                                     ysem.at[j % (2 * B3U)])

    cp_c = pltpu.make_async_copy(c_hbm, c_v, sems.at[0])
    cp_x = pltpu.make_async_copy(x_hbm, x_v, sems.at[1])
    cp_wr = pltpu.make_async_copy(wr_hbm, wr_v, sems.at[2])
    cp_wi = pltpu.make_async_copy(wi_hbm, wi_v, sems.at[3])
    cp_dfw = pltpu.make_async_copy(dfw_hbm, dfw_v, sems.at[4])
    cp_dinv = pltpu.make_async_copy(dinv_hbm, dinv_v, sems.at[5])
    cp_base = pltpu.make_async_copy(base_hbm, base_v, sems.at[6])
    cp_tw = pltpu.make_async_copy(tw_hbm, tw_v, sems.at[8])
    cp_wo = pltpu.make_async_copy(wo_hbm, wo_v, sems.at[7])

    for c in (cp_dfw, cp_base, cp_tw):
        c.start()
    for j in range(N2 // 2):
        bx_copy(j).start()

    for c in (cp_dfw, cp_base, cp_tw):
        c.wait()
    n1 = N2 // 2 // B1U

    def b1_body(i, carry):
        for u in range(B1U):
            bx_copy(i * B1U + u).wait()

        @pl.when(i == 0)
        def _():
            cp_c.start()
            cp_x.start()
            for c in w_copies(0, 0):
                c.start()

        for u in range(B1U):
            _b_stage1(i * B1U + u, xb, dfw_v, base_v, tw_v, t_s)
        return carry

    lax.fori_loop(0, n1, b1_body, 0)

    def lhs_sums(src, dst, kh):
        def body(r, carry):
            top = pl.ds(pl.multiple_of(r * SRC, SRC), SRC)
            bot = pl.ds(pl.multiple_of(HS + r * SRC, SRC), SRC)
            ops = _strassen_lhs(src[top, pl.ds(0, kh)], src[top, pl.ds(kh, kh)],
                                src[bot, pl.ds(0, kh)], src[bot, pl.ds(kh, kh)])
            for i, o in enumerate((0, 1, 4, 5, 6)):
                dst[i, top, :] = ops[o]
            return carry
        lax.fori_loop(0, HS // SRC, body, 0)

    def lhs_load(src, sums, kh):
        top, bot = pl.ds(0, HS), pl.ds(HS, HS)
        return [sums[0], sums[1], src[top, pl.ds(0, kh)], src[bot, pl.ds(kh, kh)],
                sums[2], sums[3], sums[4]]

    cp_c.wait()
    lhs_sums(c_v, cs_v, DC // 2)
    cp_x.wait()
    lhs_sums(x_v, xs_v, M // 2)

    def project_pair(slot):
        top, bot = pl.ds(0, HS), pl.ds(HS, HS)

        def half(buf, r0, n, e):
            return lambda: _unpack2(buf[slot, pl.ds(r0, n), :])[e]

        def kv(e):
            n = DC // 2
            c11, c12, c21, c22 = _strassen(lhs_load(c_v, cs_v, n),
                                           _rhs_ops(half(wk_b, 0, n, e), half(wv_b, 0, n, e),
                                                    half(wk_b, n, n, e), half(wv_b, n, n, e)))
            k_s[e, top, :] = c11.astype(bf16)
            v_s[e, top, :] = c12.astype(bf16)
            k_s[e, bot, :] = c21.astype(bf16)
            v_s[e, bot, :] = c22.astype(bf16)

        kv(0)
        n = M // 2
        c11, c12, c21, c22 = _strassen(lhs_load(x_v, xs_v, n),
                                       _rhs_ops(half(wq_b, 0, n, 0), half(wq_b, 0, n, 1),
                                                half(wq_b, n, n, 0), half(wq_b, n, n, 1)))
        q_s[0, top, :] = (c11 * QSCALE).astype(bf16)
        q_s[1, top, :] = (c12 * QSCALE).astype(bf16)
        q_s[0, bot, :] = (c21 * QSCALE).astype(bf16)
        q_s[1, bot, :] = (c22 * QSCALE).astype(bf16)
        kv(1)

    def pair_body(p, carry):
        slot = p % 2
        for c in w_copies(p, slot):
            c.wait()

        @pl.when(p + 1 < NP)
        def _():
            for c in w_copies(p + 1, 1 - slot):
                c.start()

        @pl.when(p == 1)
        def _():
            cp_wo.start()

        @pl.when(p == 4)
        def _():
            for c in (cp_wr, cp_wi, cp_dinv):
                c.start()

        project_pair(slot)
        for e in range(2):
            flags[2 * p + e] = _attn_fast(q_s.at[e], k_s.at[e], v_s.at[e], ctx_s.at[2 * p + e])
        return carry

    lax.fori_loop(0, NP, pair_body, 0)

    any_bad = jnp.max(flags[...].reshape(H * 8, 128))

    @pl.when(any_bad > 0)
    def _():
        def redo(h, carry):
            @pl.when(jnp.max(flags[h]) > 0)
            def _():
                p = h // 2
                e = h % 2
                for c in w_copies(p, 0):
                    c.start()
                for c in w_copies(p, 0):
                    c.wait()
                wq = _unpack_head(wq_b.at[0], e)
                wk = _unpack_head(wk_b.at[0], e)
                wv = _unpack_head(wv_b.at[0], e)

                def proj(r, carry):
                    rs = pl.ds(pl.multiple_of(r * 256, 256), 256)
                    cblk = c_v[rs, :]
                    k_s[0, rs, :] = jnp.dot(cblk, wk, preferred_element_type=f32).astype(bf16)
                    v_s[0, rs, :] = jnp.dot(cblk, wv, preferred_element_type=f32).astype(bf16)
                    q_s[0, rs, :] = jnp.dot(x_v[rs, :], wq, preferred_element_type=f32).astype(bf16)
                    return carry
                lax.fori_loop(0, SEQ // 256, proj, 0)
                _attn_exact(q_s.at[0], k_s.at[0], v_s.at[0], ctx_s.at[h])
            return carry
        lax.fori_loop(0, H, redo, 0)

    cp_wr.wait()
    cp_wi.wait()
    cp_wo.wait()
    n_oc = HS // ORC
    gpi = 32 // n_oc

    def oproj_body(r):
        top = pl.ds(r * ORC, ORC)
        bot = pl.ds(HS + r * ORC, ORC)
        ng = NP // OKG
        ms = [None] * 7
        for g in range(ng):
            def blk(rows, h0):
                return jnp.concatenate([ctx_s[h0 + g * OKG + i, rows, :] for i in range(OKG)], axis=1)

            def wblk(h0, c0):
                return lambda: wo_v[pl.ds(h0 + g * OKG, OKG), :, pl.ds(c0, M // 2)].reshape(
                    OKG * D, M // 2).astype(f32)
            lhs = _strassen_lhs(blk(top, 0), blk(top, NP), blk(bot, 0), blk(bot, NP))
            rhs = _rhs_ops(wblk(0, 0), wblk(0, M // 2), wblk(NP, 0), wblk(NP, M // 2))
            for i in range(7):
                t = jnp.dot(lhs[i], rhs[i](), preferred_element_type=f32)
                ms[i] = t if ms[i] is None else ms[i] + t
                if i in (1, 4):
                    idx = g * 2 + (i == 4)
                    for u in range(gpi // (2 * ng)):
                        _b_stage2(r * gpi + idx * (gpi // (2 * ng)) + u, t_s, vv_s, wr_v, wi_v)
        m1, m2, m3, m4, m5, m6, m7 = ms
        slot = r
        n = ORC // N2
        for half, (cl, cr) in enumerate(((m1 + m4 - m5 + m7, m3 + m5), (m2 + m4, m1 - m2 + m3 + m6))):
            o_st[slot, half, :, :, pl.ds(0, M // 2)] = cl.astype(bf16).reshape(n, N2, M // 2)
            o_st[slot, half, :, :, pl.ds(M // 2, M // 2)] = cr.astype(bf16).reshape(n, N2, M // 2)
        for half in range(2):
            out_copy(r, slot, half).start()

    for r in range(n_oc):
        oproj_body(r)

    cp_dinv.wait()
    n3 = N2 // 2 // B3U

    def b3_body(i, carry):
        @pl.when(i >= 2)
        def _():
            for u in range(B3U):
                y_copy((i - 2) * B3U + u).wait()

        ys = [_b_stage3(i * B3U + u, vv_s, base_v, tw_v, dinv_v) for u in range(B3U)]
        for u in range(B3U):
            y_st[(i * B3U + u) % (2 * B3U)] = ys[u]
        for u in range(B3U):
            y_copy(i * B3U + u).start()
        return carry

    lax.fori_loop(0, n3, b3_body, 0)
    for r in (n_oc - 2, n_oc - 1):
        for half in range(2):
            out_copy(r, r % 2, half).wait()
    for j in range((n3 - 2) * B3U, n3 * B3U):
        y_copy(j).wait()


@jax.jit
def pallas_concat_heads__compressed_kv_cla__spectral_gfnet__prompt_kernel(
    A_x: jax.Array,
    A_c_kv: jax.Array,
    A_w_q: jax.Array,
    A_w_uk: jax.Array,
    A_w_uv: jax.Array,
    A_w_o: jax.Array,
    B_x: jax.Array,
    B_w_r: jax.Array,
    B_w_i: jax.Array,
):
    dfw, dinv, base, tw = _dft_consts()
    hbm = pl.BlockSpec(memory_space=pltpu.HBM)
    bf16, f32, u32 = jnp.bfloat16, jnp.float32, jnp.uint32
    scratch = [
        pltpu.VMEM((SEQ, M), bf16), pltpu.VMEM((SEQ, DC), bf16),
        pltpu.VMEM((5, HS, M // 2), bf16), pltpu.VMEM((5, HS, DC // 2), bf16),
        pltpu.VMEM((2, M, D), u32), pltpu.VMEM((2, DC, D), u32), pltpu.VMEM((2, DC, D), u32),
        pltpu.VMEM((H, D, M), bf16),
        pltpu.VMEM((2, SEQ, D), bf16), pltpu.VMEM((2, SEQ, D), bf16), pltpu.VMEM((2, SEQ, D), bf16),
        pltpu.VMEM((H, SEQ, D), bf16),
        pltpu.VMEM((H, 8, 128), jnp.int32),
        pltpu.VMEM((2, 2, ORC // N2, N2, M), bf16),
        pltpu.VMEM((N2 // 2, N1, DB), u32),
        pltpu.VMEM(dfw.shape, bf16), pltpu.VMEM(dinv.shape, bf16),
        pltpu.VMEM(base.shape, f32), pltpu.VMEM(tw.shape, f32),
        pltpu.VMEM((DF, SB), bf16), pltpu.VMEM((DF, SB), bf16),
        pltpu.VMEM((N2, UR, 256), f32), pltpu.VMEM((N2, VR, 256), f32),
        pltpu.VMEM((2 * B3U, N1, DB), u32),
        pltpu.SemaphoreType.DMA((9,)), pltpu.SemaphoreType.DMA((2, 3)),
        pltpu.SemaphoreType.DMA((N2 // 2,)),
        pltpu.SemaphoreType.DMA((2, 2)), pltpu.SemaphoreType.DMA((2 * B3U,)),
    ]
    out = pl.pallas_call(
        _kernel,
        out_shape=jax.ShapeDtypeStruct((N1, N2, M + DB), bf16),
        in_specs=[hbm] * 13,
        out_specs=hbm,
        scratch_shapes=scratch,
        compiler_params=pltpu.CompilerParams(vmem_limit_bytes=126 * 2 ** 20),
    )(A_x.reshape(SEQ, M), A_c_kv.reshape(SEQ, DC), A_w_q, A_w_uk, A_w_uv, A_w_o,
      B_x.reshape(N1, N2, DB), B_w_r.T, B_w_i.T, dfw, dinv, base, tw)
    return out.reshape(1, SEQ, M + DB)
```

```python
import functools
import math

import jax
import jax.numpy as jnp
import jax.experimental.pallas as pl
import jax.experimental.pallas.tpu as pltpu
import ml_dtypes
import numpy as np
from jax import lax

SEQ = 2048
D = 128
H = 32
M = 1024
DC = 512
SB = 2048
DB = 1024
DF = DB // 2 + 1
N1 = 128
N2 = 16
UR = 528
VR = 512
NT = (((1,), (1,)), ((), ()))
QSCALE = (D ** -0.5) * math.log2(math.e)
L_LO = 2.0 ** -30
L_HI = 2.0 ** 30
HI16 = 0xFFFF0000
BAL = 4.0
BQ = BK = 512


@functools.lru_cache(maxsize=None)
def _dft_consts():
    th = 2 * np.pi / DB
    d = np.arange(256, dtype=np.float64) + 0.5
    m = np.arange(256, dtype=np.float64)
    fe, fo = 2 * m, 2 * m + 1
    sny = np.zeros((16, 256))
    sny[0] = -np.sin(th * 512 * d)
    dfw = np.concatenate([np.cos(th * np.outer(fe, d)), np.cos(th * np.outer(fo, d)),
                          -np.sin(th * np.outer(fe, d)), sny, -np.sin(th * np.outer(fo, d))], 0)
    cfe = np.full(256, 2.0 / DB)
    cfe[0] = 1.0 / DB
    cfo = np.full(256, 2.0 / DB)
    gse = cfe[:, None] * np.sin(th * np.outer(fe, d))
    gse[0] = (1.0 / DB) * np.sin(th * 512 * d)
    dinv = np.stack([cfe[:, None] * np.cos(th * np.outer(fe, d)),
                     cfo[:, None] * np.cos(th * np.outer(fo, d)),
                     gse, cfo[:, None] * np.sin(th * np.outer(fo, d))], 0)
    n1 = np.arange(N1)[:, None]
    k1 = np.arange(N1)[None, :]
    base = np.stack([np.cos(2 * np.pi * n1 * k1 / N1), -np.sin(2 * np.pi * n1 * k1 / N1)], 0)
    n2 = np.arange(N2)[:, None]
    tw = np.stack([np.cos(2 * np.pi * n2 * k1 / SB), -np.sin(2 * np.pi * n2 * k1 / SB)], 0)
    tw = np.repeat(tw[:, :, None, :], 8, axis=2)
    bf = ml_dtypes.bfloat16
    return (np.asarray(dfw, dtype=np.float32).astype(bf), np.asarray(dinv, dtype=np.float32).astype(bf),
            base.astype(np.float32), tw.astype(np.float32))


def _cmul_const(xr, xi, ang):
    c, s = math.cos(ang), math.sin(ang)
    eps = 1e-9
    if abs(s) < eps:
        return (xr, xi) if c > 0 else (-xr, -xi)
    if abs(c) < eps:
        return (-xi, xr) if s > 0 else (xi, -xr)
    if abs(abs(c) - abs(s)) < eps:
        if c * s > 0:
            return (xr - xi) * c, (xr + xi) * c
        return (xr + xi) * c, (xi - xr) * c
    return xr * c - xi * s, xr * s + xi * c


def _fft(xs, sign):
    n = len(xs)
    if n == 1:
        return xs
    if n == 2:
        (ar, ai), (br, bi) = xs
        return [(ar + br, ai + bi), (ar - br, ai - bi)]
    if n == 4:
        (ar, ai), (br, bi), (cr, ci), (dr, di) = xs
        t0r, t0i = ar + cr, ai + ci
        t1r, t1i = ar - cr, ai - ci
        t2r, t2i = br + dr, bi + di
        t3r, t3i = br - dr, bi - di
        if sign > 0:
            return [(t0r + t2r, t0i + t2i), (t1r - t3i, t1i + t3r),
                    (t0r - t2r, t0i - t2i), (t1r + t3i, t1i - t3r)]
        return [(t0r + t2r, t0i + t2i), (t1r + t3i, t1i - t3r),
                (t0r - t2r, t0i - t2i), (t1r - t3i, t1i + t3r)]
    ev = _fft(xs[0::2], sign)
    od = _fft(xs[1::2], sign)
    out = [None] * n
    for k in range(n // 2):
        er, ei = ev[k]
        if k * 4 == n:
            o_r, o_i = od[k]
            if sign > 0:
                out[k] = (er - o_i, ei + o_r)
                out[k + n // 2] = (er + o_i, ei - o_r)
            else:
                out[k] = (er + o_i, ei - o_r)
                out[k + n // 2] = (er - o_i, ei + o_r)
        else:
            tr, ti = _cmul_const(od[k][0], od[k][1], sign * 2 * math.pi * k / n)
            out[k] = (er + tr, ei + ti)
            out[k + n // 2] = (er - tr, ei - ti)
    return out


def _unpack_head(wbuf, e):
    sh = (16 * (1 - e)).astype(jnp.uint32)
    w = pltpu.bitcast((wbuf[...] << sh) & jnp.uint32(HI16), jnp.float32)
    return w.astype(jnp.bfloat16)


def _strassen_lhs(f11, f12, f21, f22):
    bf = jnp.bfloat16
    return [(f11 + f22).astype(bf), (f21 + f22).astype(bf), f11.astype(bf), f22.astype(bf),
            (f11 + f12).astype(bf), (f21 - f11).astype(bf), (f12 - f22).astype(bf)]


def _unbalanced(n11, n12, n21, n22):
    hi = jnp.maximum(jnp.maximum(n11, n12), jnp.maximum(n21, n22))
    lo = jnp.minimum(jnp.minimum(n11, n12), jnp.minimum(n21, n22))
    return jnp.where(hi <= BAL * lo, 0, 1).astype(jnp.int32)


def _fold8(a, op):
    r = a[0:8]
    for i in range(1, a.shape[0] // 8):
        r = op(r, a[i * 8:(i + 1) * 8])
    return r


def _rows_to_bf16(even, odd):
    return pltpu.bitcast(pltpu.pack_elementwise([even, odd], packed_dtype=jnp.bfloat16), jnp.bfloat16)


def _attn_plan(qi, bq, bk, stair):
    r0 = qi * bq
    steps = []
    c = 0
    while c + bk <= r0:
        steps.append((0, c, bk))
        c += bk
    if c < r0:
        steps.append((0, c, r0 - c))
    diag = [(t * stair, r0 + t * stair, stair) for t in range(bq // stair)]
    return diag + steps


def _attn_fast(q_ref, k_ref, v_ref, o_ref, n_ref, bq=BQ, bk=BK, stair=128):
    R = 128
    row = lax.broadcasted_iota(jnp.int32, (R, 128), 0)
    col = lax.broadcasted_iota(jnp.int32, (R, 128), 1)
    tri = col <= row
    bad = jnp.zeros((8, 128), jnp.int32)
    for qi in range(SEQ // bq):
        r0 = qi * bq
        nsub = bq // R
        acc = [None] * nsub
        lv = [None] * nsub
        for (roff, c0, clen) in _attn_plan(qi, bq, bk, stair):
            mr = bq - roff
            q = q_ref[pl.ds(r0 + roff, mr), :]
            k = k_ref[pl.ds(c0, clen), :]
            v = v_ref[pl.ds(c0, clen), :]
            s = lax.dot_general(q, k, NT, preferred_element_type=jnp.float32)
            p = jnp.exp2(s)
            if c0 + clen - 1 > r0 + roff:
                rows = []
                for a in range(mr // R):
                    ra = r0 + roff + a * R
                    cols = []
                    for b in range(clen // 128):
                        cb = c0 + b * 128
                        t = p[a * R:(a + 1) * R, b * 128:(b + 1) * 128]
                        if cb == ra:
                            t = jnp.where(tri, t, 0.0)
                        elif cb > ra:
                            t = jnp.zeros_like(t)
                        cols.append(t)
                    rows.append(jnp.concatenate(cols, axis=1) if len(cols) > 1 else cols[0])
                p = jnp.concatenate(rows, axis=0) if len(rows) > 1 else rows[0]
            pv = jnp.dot(p.astype(jnp.bfloat16), v, preferred_element_type=jnp.float32)
            for a in range(mr // R):
                ia = roff // R + a
                pa = p[a * R:(a + 1) * R, :]
                ps = pa[:, 0:128]
                for b in range(1, clen // 128):
                    ps = ps + pa[:, b * 128:(b + 1) * 128]
                lv[ia] = ps if lv[ia] is None else lv[ia] + ps
                t = pv[a * R:(a + 1) * R, :]
                acc[ia] = t if acc[ia] is None else acc[ia] + t
        for a in range(nsub):
            l = jnp.sum(lv[a], axis=-1, keepdims=True)
            o = acc[a] * (1.0 / l)
            ok = (l >= L_LO) & (l <= L_HI) & (jnp.abs(o) <= 3.0e38)
            nb = jnp.where(ok, 0, 1).astype(jnp.int32)
            for i in range(R // 8):
                bad = jnp.maximum(bad, nb[i * 8:(i + 1) * 8, :])
            o_ref[pl.ds(r0 + a * R, R), :] = o.astype(o_ref.dtype)
            n_ref[pl.ds(r0 + a * R, R), :] += o * o
    return bad


def _attn_exact(q_ref, k_ref, v_ref, o_ref, bq=256, bk=256):
    scale = D ** -0.5

    def q_body(qi, carry):
        rs = pl.ds(pl.multiple_of(qi * bq, bq), bq)
        q = q_ref[rs, :]

        def k_body(kj, st):
            m, l, acc = st
            ks = pl.ds(pl.multiple_of(kj * bk, bk), bk)
            s = lax.dot_general(q, k_ref[ks, :], NT, preferred_element_type=jnp.float32) * scale
            row = lax.broadcasted_iota(jnp.int32, (bq, bk), 0) + qi * bq
            col = lax.broadcasted_iota(jnp.int32, (bq, bk), 1) + kj * bk
            s = jnp.where(col <= row, s, -1e9)
            m_new = jnp.maximum(m, jnp.max(s, axis=-1, keepdims=True))
            p = jnp.exp(s - m_new)
            alpha = jnp.exp(m - m_new)
            l = alpha * l + jnp.sum(p, axis=-1, keepdims=True)
            acc = alpha * acc + jnp.dot(p.astype(jnp.bfloat16), v_ref[ks, :],
                                        preferred_element_type=jnp.float32)
            return m_new, l, acc

        init = (jnp.full((bq, 1), -jnp.inf, jnp.float32), jnp.zeros((bq, 1), jnp.float32),
                jnp.zeros((bq, D), jnp.float32))
        m, l, acc = lax.fori_loop(0, SEQ // bk, k_body, init)
        o_ref[rs, :] = (acc / l).astype(o_ref.dtype)
        return carry

    lax.fori_loop(0, SEQ // bq, q_body, 0)


def _unpack2(u):
    return (pltpu.bitcast(u << 16, jnp.float32), pltpu.bitcast(u & jnp.uint32(HI16), jnp.float32))


def _s_matrix(n2, base_ref, tw_ref):
    fr, fi = [], []
    for r in range(N1 // 8):
        br = base_ref[0, pl.ds(r * 8, 8), :]
        bi = base_ref[1, pl.ds(r * 8, 8), :]
        tr = tw_ref[0, n2]
        ti = tw_ref[1, n2]
        fr.append(br * tr - bi * ti)
        fi.append(br * ti + bi * tr)
    return jnp.concatenate(fr, axis=0), jnp.concatenate(fi, axis=0)


def _b_stage1(j, xb, dfw_ref, base_ref, tw_ref, tv):
    bf = jnp.bfloat16
    ridx = 127 - lax.broadcasted_iota(jnp.int32, (N1, 128), 1)
    q0, q1r, q2, q3r = [], [], [], []
    for t in range(2):
        q0.append(_unpack2(xb[j, :, pl.ds(t * 128, 128)]))
        q1r.append(_unpack2(jnp.take_along_axis(xb[j, :, pl.ds((3 - t) * 128, 128)], ridx, axis=1)))
        q2.append(_unpack2(xb[j, :, pl.ds((4 + t) * 128, 128)]))
        q3r.append(_unpack2(jnp.take_along_axis(xb[j, :, pl.ds((7 - t) * 128, 128)], ridx, axis=1)))
    for e in range(2):
        n2 = 2 * j + e
        ee, eo, oe, oo = [], [], [], []
        for t in range(2):
            x0, r1, x2, r3 = q0[t][e], q1r[t][e], q2[t][e], q3r[t][e]
            a = x0 + r3
            b = x0 - r3
            c = r1 + x2
            dd = r1 - x2
            ee.append((a + c).astype(jnp.bfloat16))
            eo.append((a - c).astype(jnp.bfloat16))
            oe.append((b - dd).astype(jnp.bfloat16))
            oo.append((b + dd).astype(jnp.bfloat16))
        ee, eo, oe, oo = (jnp.concatenate(z, axis=1) for z in (ee, eo, oe, oo))
        ur_e = lax.dot_general(dfw_ref[pl.ds(0, 256), :], ee, NT, preferred_element_type=jnp.float32)
        ur_o = lax.dot_general(dfw_ref[pl.ds(256, 256), :], eo, NT, preferred_element_type=jnp.float32)
        ui_en = lax.dot_general(dfw_ref[pl.ds(512, 272), :], oe, NT, preferred_element_type=jnp.float32)
        ui_o = lax.dot_general(dfw_ref[pl.ds(784, 256), :], oo, NT, preferred_element_type=jnp.float32)
        ur = jnp.concatenate([ur_e, ur_o, jnp.zeros((16, 128), jnp.float32)], axis=0)
        ui = jnp.concatenate([ui_en[:256], ui_o, ui_en[256:]], axis=0)
        fr, fi = _s_matrix(n2, base_ref, tw_ref)
        k1 = jnp.dot(ur.astype(bf), fr.astype(bf), preferred_element_type=jnp.float32)
        k2 = jnp.dot(ui.astype(bf), fi.astype(bf), preferred_element_type=jnp.float32)
        k3 = jnp.dot((ur + ui).astype(bf), (fr + fi).astype(bf), preferred_element_type=jnp.float32)
        tv[n2, pl.ds(0, UR), pl.ds(0, 128)] = k1 - k2
        tv[n2, pl.ds(0, UR), pl.ds(128, 128)] = k3 - k1 - k2


def _b_filtered(r0, t_s, w_of):
    xs = [(t_s[n2, pl.ds(r0, 8), pl.ds(0, 128)], t_s[n2, pl.ds(r0, 8), pl.ds(128, 128)])
          for n2 in range(N2)]
    zs = []
    for k2, (xr, xi) in enumerate(_fft(xs, -1)):
        wr, wi = w_of(pl.ds(k2 * 128, 128))
        zs.append((xr * wr - xi * wi, xr * wi + xi * wr))
    return zs


def _b_stage2(g, t_s, v_s, wr_v, wi_v):
    for kind in (0, 1):
        r0 = kind * 256 + g * 8

        def w_of(cs):
            return tuple(_unpack2(pltpu.bitcast(w[pl.ds(g * 16, 16), cs], jnp.uint32))[kind]
                         for w in (wr_v, wi_v))
        zs = _b_filtered(r0, t_s, w_of)
        if g == 0 and kind == 0:
            def w_ny(cs):
                return tuple(jnp.broadcast_to(w[pl.ds(512, 1), cs].astype(jnp.float32), (8, 128))
                             for w in (wr_v, wi_v))
            ns = _b_filtered(512, t_s, w_ny)
            lane = lax.broadcasted_iota(jnp.int32, (8, 128), 1)
            row = lax.broadcasted_iota(jnp.int32, (8, 128), 0)
            idx = (128 - lane) % 128
            da = [z[0] - n[0] for z, n in zip(zs, ns)]
            db = [n[1] - z[1] for z, n in zip(zs, ns)]

            def rev(x, k2):
                return jnp.where(lane == 0, x[(N2 - k2) % N2],
                                 jnp.take_along_axis(x[N2 - 1 - k2], idx, axis=1))
            zs = [(jnp.where(row == 0, 0.5 * (z[0] + n[0] + rev(da, k2)), z[0]),
                   jnp.where(row == 0, 0.5 * (z[1] + n[1] + rev(db, k2)), z[1]))
                  for k2, (z, n) in enumerate(zip(zs, ns))]
        vs = _fft(zs, +1)
        for n2 in range(N2):
            v_s[n2, pl.ds(r0, 8), pl.ds(0, 128)] = vs[n2][0]
            v_s[n2, pl.ds(r0, 8), pl.ds(128, 128)] = vs[n2][1]


def _b_stage3(j, tv, base_ref, tw_ref, dinv_ref):
    bf = jnp.bfloat16
    ridx = 127 - lax.broadcasted_iota(jnp.int32, (N1, 128), 1)
    zr, zi = [], []
    for e in range(2):
        n2 = 2 * j + e
        vr = tv[n2, :, pl.ds(0, 128)]
        vi = tv[n2, :, pl.ds(128, 128)]
        fr, fi = _s_matrix(n2, base_ref, tw_ref)
        gr, gi = fr * (1.0 / SB), fi * (-1.0 / SB)
        k1 = lax.dot_general(gr.astype(bf), vr.astype(bf), NT, preferred_element_type=jnp.float32)
        k2 = lax.dot_general(gi.astype(bf), vi.astype(bf), NT, preferred_element_type=jnp.float32)
        k3 = lax.dot_general((gr + gi).astype(bf), (vr + vi).astype(bf), NT,
                             preferred_element_type=jnp.float32)
        zr.append((k1 - k2).astype(bf))
        zi.append((k3 - k1 - k2).astype(bf))
    zr = jnp.concatenate(zr, axis=0)
    zi = jnp.concatenate(zi, axis=0)
    pe = jnp.dot(zr[:, :256], dinv_ref[0], preferred_element_type=jnp.float32)
    po = jnp.dot(zr[:, 256:], dinv_ref[1], preferred_element_type=jnp.float32)
    qe = jnp.dot(zi[:, :256], dinv_ref[2], preferred_element_type=jnp.float32)
    qo = jnp.dot(zi[:, 256:], dinv_ref[3], preferred_element_type=jnp.float32)
    ps, pd, qs, qd = pe + po, pe - po, qe + qo, qe - qo
    y0, y1r, y2, y3r = ps - qs, pd + qd, pd - qd, ps + qs

    def pk(y, t):
        return pltpu.pack_elementwise([y[:128, t * 128:(t + 1) * 128], y[128:, t * 128:(t + 1) * 128]],
                                      packed_dtype=jnp.bfloat16)

    outs = [None] * 8
    for t in range(2):
        outs[t] = pk(y0, t)
        outs[3 - t] = jnp.take_along_axis(pk(y1r, t), ridx, axis=1)
        outs[4 + t] = pk(y2, t)
        outs[7 - t] = jnp.take_along_axis(pk(y3r, t), ridx, axis=1)
    return jnp.concatenate(outs, axis=1)


HS = SEQ // 2
ORC = 512
OKG = 2
B1U = 2
B3U = 2
NP = H // 2

SRC = 32


def _rhs_ops(b11, b12, b21, b22):
    bf = jnp.bfloat16
    return [lambda: (b11() + b22()).astype(bf), lambda: b11().astype(bf),
            lambda: (b12() - b22()).astype(bf), lambda: (b21() - b11()).astype(bf),
            lambda: b22().astype(bf), lambda: (b11() + b12()).astype(bf),
            lambda: (b21() + b22()).astype(bf)]


def _strassen(lhs, rhs):
    m1, m2, m3, m4, m5, m6, m7 = (jnp.dot(a, b(), preferred_element_type=jnp.float32)
                                  for a, b in zip(lhs, rhs))
    return m1 + m4 - m5 + m7, m3 + m5, m2 + m4, m1 - m2 + m3 + m6


def _kernel(x_hbm, c_hbm, wq_hbm, wk_hbm, wv_hbm, wo_hbm, bx_hbm, wr_hbm, wi_hbm,
            dfw_hbm, dinv_hbm, base_hbm, tw_hbm, o_hbm,
            x_v, c_v, xs_v, cs_v, wq_b, wk_b, wv_b, wo_v, q_s, k_s, v_s, ctx_s, nrm_s, sq_s, flags, wflags, o_st,
            xb, dfw_v, dinv_v, base_v, tw_v, wr_v, wi_v, t_s, vv_s, y_st,
            sems, wsem, xsem, osem, ysem):
    f32, bf16 = jnp.float32, jnp.bfloat16
    wq_u = wq_hbm.bitcast(jnp.uint32)
    wk_u = wk_hbm.bitcast(jnp.uint32)
    wv_u = wv_hbm.bitcast(jnp.uint32)
    bx_u = bx_hbm.bitcast(jnp.uint32)
    o_u = o_hbm.bitcast(jnp.uint32)

    def w_copies(p, slot):
        return [pltpu.make_async_copy(wq_u.at[:, p, :], wq_b.at[slot], wsem.at[slot, 0]),
                pltpu.make_async_copy(wk_u.at[:, p, :], wk_b.at[slot], wsem.at[slot, 1]),
                pltpu.make_async_copy(wv_u.at[:, p, :], wv_b.at[slot], wsem.at[slot, 2])]

    def bx_copy(j):
        return pltpu.make_async_copy(bx_u.at[:, j, :], xb.at[j], xsem.at[j])

    def out_copy(r):
        n = 2 * ORC // N2
        return pltpu.make_async_copy(o_st.at[r], o_hbm.at[pl.ds(r * n, n), :, pl.ds(0, M)], osem.at[r])

    def y_copy(j):
        return pltpu.make_async_copy(y_st.at[j % (2 * B3U)], o_u.at[:, j, pl.ds(M, DB)],
                                     ysem.at[j % (2 * B3U)])

    cp_c = pltpu.make_async_copy(c_hbm, c_v, sems.at[0])
    cp_x = pltpu.make_async_copy(x_hbm, x_v, sems.at[1])
    cp_wr = pltpu.make_async_copy(wr_hbm, wr_v, sems.at[2])
    cp_wi = pltpu.make_async_copy(wi_hbm, wi_v, sems.at[3])
    cp_dfw = pltpu.make_async_copy(dfw_hbm, dfw_v, sems.at[4])
    cp_dinv = pltpu.make_async_copy(dinv_hbm, dinv_v, sems.at[5])
    cp_base = pltpu.make_async_copy(base_hbm, base_v, sems.at[6])
    cp_tw = pltpu.make_async_copy(tw_hbm, tw_v, sems.at[8])
    cp_wo = pltpu.make_async_copy(wo_hbm, wo_v, sems.at[7])

    for c in (cp_dfw, cp_base, cp_tw):
        c.start()
    for j in range(N2 // 2):
        bx_copy(j).start()

    for c in (cp_dfw, cp_base, cp_tw):
        c.wait()
    n1 = N2 // 2 // B1U

    def b1_body(i, carry):
        for u in range(B1U):
            bx_copy(i * B1U + u).wait()

        @pl.when(i == 0)
        def _():
            cp_c.start()
            cp_x.start()
            for c in w_copies(0, 0):
                c.start()

        for u in range(B1U):
            _b_stage1(i * B1U + u, xb, dfw_v, base_v, tw_v, t_s)
        return carry

    lax.fori_loop(0, n1, b1_body, 0)

    def lane_fold(a):
        r = a[:, 0:128]
        for i in range(1, a.shape[1] // 128):
            r = r + a[:, i * 128:(i + 1) * 128]
        return r

    def balance(load, n, rows):
        bad = jnp.zeros((8, 1), jnp.int32)
        for r in range(0, n, rows):
            u = _unbalanced(*[jnp.sum(load(i, pl.ds(r, rows)), axis=1, keepdims=True) for i in range(4)])
            bad = jnp.maximum(bad, _fold8(u, jnp.maximum))
        return jnp.max(bad)

    def lhs_sums(src, dst, kh):
        def body(r, carry):
            ev, od = _unpack2(pltpu.bitcast(src[pl.ds(pl.multiple_of(r * SRC, SRC), SRC), :], jnp.uint32))
            blocks = (ev[:, :kh], ev[:, kh:], od[:, :kh], od[:, kh:])
            rows = pl.ds(pl.multiple_of(r * (SRC // 2), SRC // 2), SRC // 2)
            for i, o in enumerate(_strassen_lhs(*blocks)):
                dst[i, rows, :] = o
            for i, f in enumerate(blocks):
                sq_s[i, rows, :] = lane_fold(f * f)
            return carry
        lax.fori_loop(0, SEQ // SRC, body, 0)
        return balance(lambda i, rows: sq_s[i, rows, :], HS, 128)

    cp_c.wait()
    bad_c = lhs_sums(c_v, cs_v, DC // 2)
    cp_x.wait()
    bad_x = lhs_sums(x_v, xs_v, M // 2)
    nrm_s[...] = jnp.zeros(nrm_s.shape, f32)

    def project_pair(slot, p):
        def project(lhs, wbuf, out_ref, scale):
            n = lhs.shape[2]

            def blk(r0, e):
                return lambda: _unpack2(wbuf[slot, pl.ds(r0, n), :])[e]
            blocks = (blk(0, 0), blk(0, 1), blk(n, 0), blk(n, 1))
            c11, c12, c21, c22 = _strassen([lhs[i] for i in range(7)], _rhs_ops(*blocks))
            if scale is not None:
                c11, c12, c21, c22 = (c * scale for c in (c11, c12, c21, c22))
            out_ref[0] = _rows_to_bf16(c11, c21)
            out_ref[1] = _rows_to_bf16(c12, c22)
            nrm = [jnp.sum(_fold8(w * w, jnp.add), axis=0, keepdims=True) for w in (b() for b in blocks)]
            return _unbalanced(*nrm)

        bad = project(cs_v, wk_b, k_s, None)
        bad = jnp.maximum(bad, project(xs_v, wq_b, q_s, QSCALE))
        bad = jnp.maximum(bad, project(cs_v, wv_b, v_s, None))
        wflags[p] = jnp.broadcast_to(bad, (8, 128))

    def pair_body(p, carry):
        slot = p % 2
        for c in w_copies(p, slot):
            c.wait()

        @pl.when(p + 1 < NP)
        def _():
            for c in w_copies(p + 1, 1 - slot):
                c.start()

        @pl.when(p == 1)
        def _():
            cp_wo.start()

        @pl.when(p == 4)
        def _():
            for c in (cp_wr, cp_wi, cp_dinv):
                c.start()

        project_pair(slot, p)
        for e in range(2):
            flags[2 * p + e] = _attn_fast(q_s.at[e], k_s.at[e], v_s.at[e], ctx_s.at[2 * p + e],
                                          nrm_s.at[p // (NP // 2)])
        return carry

    lax.fori_loop(0, NP, pair_body, 0)

    any_bad = jnp.maximum(jnp.maximum(jnp.max(flags[...].reshape(H * 8, 128)),
                                      jnp.max(wflags[...].reshape(NP * 8, 128))),
                          jnp.maximum(bad_c, bad_x))

    @pl.when(any_bad > 0)
    def _():
        nrm_s[...] = jnp.zeros(nrm_s.shape, f32)

        def redo(h, carry):
            p = h // 2
            e = h % 2
            for c in w_copies(p, 0):
                c.start()
            for c in w_copies(p, 0):
                c.wait()
            wq = _unpack_head(wq_b.at[0], e)
            wk = _unpack_head(wk_b.at[0], e)
            wv = _unpack_head(wv_b.at[0], e)

            def proj(r, carry):
                rs = pl.ds(pl.multiple_of(r * 256, 256), 256)
                cblk = c_v[rs, :]
                k_s[0, rs, :] = jnp.dot(cblk, wk, preferred_element_type=f32).astype(bf16)
                v_s[0, rs, :] = jnp.dot(cblk, wv, preferred_element_type=f32).astype(bf16)
                q_s[0, rs, :] = jnp.dot(x_v[rs, :], wq, preferred_element_type=f32).astype(bf16)
                return carry
            lax.fori_loop(0, SEQ // 256, proj, 0)
            _attn_exact(q_s.at[0], k_s.at[0], v_s.at[0], ctx_s.at[h])
            o = ctx_s[h].astype(f32)
            nrm_s[h // NP] += o * o
            return carry
        lax.fori_loop(0, H, redo, 0)

    cp_wr.wait()
    cp_wi.wait()
    cp_wo.wait()
    n_oc = HS // ORC

    for g in range(32):
        _b_stage2(g, t_s, vv_s, wr_v, wi_v)

    bad_o = balance(lambda i, rows: nrm_s[i % 2, pl.ds(2 * rows.start + i // 2, rows.size, stride=2), :], HS, 128)
    wn = [jnp.zeros((8, M // 2), f32) for _ in range(4)]

    def oproj_body(r):
        rows = pl.ds(r * 2 * ORC, 2 * ORC)
        ng = NP // OKG
        ms = [None] * 7
        for g in range(ng):
            def blk(h0):
                return _unpack2(jnp.concatenate(
                    [pltpu.bitcast(ctx_s[h0 + g * OKG + i, rows, :], jnp.uint32) for i in range(OKG)], axis=1))

            def wblk(h0, c0):
                return lambda: wo_v[pl.ds(h0 + g * OKG, OKG), :, pl.ds(c0, M // 2)].reshape(
                    OKG * D, M // 2).astype(f32)
            f11, f21 = blk(0)
            f12, f22 = blk(NP)
            lhs = _strassen_lhs(f11, f12, f21, f22)
            wb = tuple(functools.lru_cache(maxsize=None)(f) if r == 0 else f
                       for f in (wblk(0, 0), wblk(0, M // 2), wblk(NP, 0), wblk(NP, M // 2)))
            rhs = _rhs_ops(*wb)
            if r == 0:
                for i in range(4):
                    w = wb[i]()
                    wn[i] = wn[i] + _fold8(w * w, jnp.add)
            for i in range(7):
                t = jnp.dot(lhs[i], rhs[i](), preferred_element_type=f32)
                ms[i] = t if ms[i] is None else ms[i] + t
        m1, m2, m3, m4, m5, m6, m7 = ms
        n = 2 * ORC // N2
        o_st[r, :, :, pl.ds(0, M // 2)] = _rows_to_bf16(m1 + m4 - m5 + m7, m2 + m4).reshape(n, N2, M // 2)
        o_st[r, :, :, pl.ds(M // 2, M // 2)] = _rows_to_bf16(m3 + m5, m1 - m2 + m3 + m6).reshape(n, N2, M // 2)

    def oproj_plain(r, carry):
        rs = pl.ds(pl.multiple_of(r * 128, 128), 128)

        def hsum(h, acc):
            return acc + jnp.dot(ctx_s[h, rs, :], wo_v[h], preferred_element_type=f32)
        acc = lax.fori_loop(0, H, hsum, jnp.zeros((128, M), f32))
        n = 128 // N2
        o_st[r // (2 * ORC // 128), pl.ds((r % (2 * ORC // 128)) * n, n)] = acc.astype(bf16).reshape(n, N2, M)
        return carry

    for r in range(n_oc):
        oproj_body(r)
    bad_w = jnp.max(_unbalanced(*[jnp.sum(n, axis=0, keepdims=True) for n in wn]))

    @pl.when(jnp.maximum(bad_o, bad_w) > 0)
    def _():
        lax.fori_loop(0, SEQ // 128, oproj_plain, 0)

    for r in range(n_oc):
        out_copy(r).start()

    cp_dinv.wait()
    n3 = N2 // 2 // B3U

    def b3_body(i, carry):
        @pl.when(i >= 2)
        def _():
            for u in range(B3U):
                y_copy((i - 2) * B3U + u).wait()

        ys = [_b_stage3(i * B3U + u, vv_s, base_v, tw_v, dinv_v) for u in range(B3U)]
        for u in range(B3U):
            y_st[(i * B3U + u) % (2 * B3U)] = ys[u]
        for u in range(B3U):
            y_copy(i * B3U + u).start()
        return carry

    lax.fori_loop(0, n3, b3_body, 0)
    for r in range(n_oc):
        out_copy(r).wait()
    for j in range((n3 - 2) * B3U, n3 * B3U):
        y_copy(j).wait()


@jax.jit
def pallas_concat_heads__compressed_kv_cla__spectral_gfnet__prompt_kernel(
    A_x: jax.Array,
    A_c_kv: jax.Array,
    A_w_q: jax.Array,
    A_w_uk: jax.Array,
    A_w_uv: jax.Array,
    A_w_o: jax.Array,
    B_x: jax.Array,
    B_w_r: jax.Array,
    B_w_i: jax.Array,
):
    dfw, dinv, base, tw = _dft_consts()
    hbm = pl.BlockSpec(memory_space=pltpu.HBM)
    bf16, f32, u32 = jnp.bfloat16, jnp.float32, jnp.uint32
    scratch = [
        pltpu.VMEM((SEQ, M), bf16), pltpu.VMEM((SEQ, DC), bf16),
        pltpu.VMEM((7, HS, M // 2), bf16), pltpu.VMEM((7, HS, DC // 2), bf16),
        pltpu.VMEM((2, M, D), u32), pltpu.VMEM((2, DC, D), u32), pltpu.VMEM((2, DC, D), u32),
        pltpu.VMEM((H, D, M), bf16),
        pltpu.VMEM((2, SEQ, D), bf16), pltpu.VMEM((2, SEQ, D), bf16), pltpu.VMEM((2, SEQ, D), bf16),
        pltpu.VMEM((H, SEQ, D), bf16),
        pltpu.VMEM((2, SEQ, D), f32), pltpu.VMEM((4, HS, 128), f32),
        pltpu.VMEM((H, 8, 128), jnp.int32), pltpu.VMEM((NP, 8, 128), jnp.int32),
        pltpu.VMEM((HS // ORC, 2 * ORC // N2, N2, M), bf16),
        pltpu.VMEM((N2 // 2, N1, DB), u32),
        pltpu.VMEM(dfw.shape, bf16), pltpu.VMEM(dinv.shape, bf16),
        pltpu.VMEM(base.shape, f32), pltpu.VMEM(tw.shape, f32),
        pltpu.VMEM((DF, SB), bf16), pltpu.VMEM((DF, SB), bf16),
        pltpu.VMEM((N2, UR, 256), f32), pltpu.VMEM((N2, VR, 256), f32),
        pltpu.VMEM((2 * B3U, N1, DB), u32),
        pltpu.SemaphoreType.DMA((9,)), pltpu.SemaphoreType.DMA((2, 3)),
        pltpu.SemaphoreType.DMA((N2 // 2,)),
        pltpu.SemaphoreType.DMA((HS // ORC,)), pltpu.SemaphoreType.DMA((2 * B3U,)),
    ]
    out = pl.pallas_call(
        _kernel,
        out_shape=jax.ShapeDtypeStruct((N1, N2, M + DB), bf16),
        in_specs=[hbm] * 13,
        out_specs=hbm,
        scratch_shapes=scratch,
        compiler_params=pltpu.CompilerParams(vmem_limit_bytes=126 * 2 ** 20),
    )(A_x.reshape(SEQ, M), A_c_kv.reshape(SEQ, DC), A_w_q, A_w_uk, A_w_uv, A_w_o,
      B_x.reshape(N1, N2, DB), B_w_r.T, B_w_i.T, dfw, dinv, base, tw)
    return out.reshape(1, SEQ, M + DB)
```
